```python
import jax
import jax.numpy as jnp

def _softmax(x, axis=-1):
    return jax.nn.softmax(x, axis=axis)
def _gelu(x):
    return jax.nn.gelu(x, approximate=True)
def _silu(x):
    return jax.nn.silu(x)
def _sigmoid(x):
    return jax.nn.sigmoid(x)
def _layernorm(x, axis=-1, eps=1e-5):
    m = jnp.mean(x, axis=axis, keepdims=True)
    v = jnp.var(x, axis=axis, keepdims=True)
    return (x - m) / jnp.sqrt(v + eps)
def _scatter_add(tgt, idx, src, axis=0):
    return tgt.at[idx].add(src)
def _segment_sum(src, seg, n):
    return jax.ops.segment_sum(src, seg, n)
class _Rng:
    def __init__(self, key):
        self._k = key
    def _next(self):
        self._k, sub = jax.random.split(self._k)
        return sub
    def normal(self, shape):
        return jax.random.normal(self._next(), shape, dtype=jnp.bfloat16)
    def randint(self, lo, hi, shape):
        return jax.random.randint(self._next(), shape, lo, hi, dtype=jnp.int32)
    def uniform(self, shape, lo=0.0, hi=1.0):
        return jax.random.uniform(self._next(), shape, jnp.bfloat16, lo, hi)
    def permutation(self, n):
        return jax.random.permutation(self._next(), n)


kernel_name = 'sequential_preLN__sliding_block_cached__glu_gated_swiglu__decode'

def setup_inputs():
    _rng = _Rng(jax.random.key(int.from_bytes(__import__("os").urandom(4), "little")))
    _w = (lambda a: (lambda t: t.astype(jnp.bfloat16) if jnp.issubdtype(t.dtype, jnp.floating) else t)(jnp.asarray(a)))
    def _A_setup():
        B, Sq, D = 1, 1, 640
        Hq, Hkv, Sk, Dh = 32, 32, 32768, 192
        assert Hq % Hkv == 0, (Hq, Hkv)
        return {
            "x": _w((lambda *s: _rng.normal(s) * 0.05)(B, Sq, D)),
            "k_cache": _w((lambda *s: _rng.normal(s) * 0.05)(B, Hkv, Sk, Dh)),
            "v_cache": _w((lambda *s: _rng.normal(s) * 0.05)(B, Hkv, Sk, Dh)),
            "wq": _w((lambda *s: _rng.normal(s) * 0.05)(D, Hq * Dh) * (D ** -0.5)),
            "wo": _w((lambda *s: _rng.normal(s) * 0.05)(Hq * Dh, D) * ((Hq * Dh) ** -0.5)),
        }
    _A_in = _A_setup()

    def _B_setup():
        B, S, D, F = 1, 1, 640, 1536
        return {
            "x": _w((lambda *s: _rng.normal(s) * 0.05)(B, S, D)),
            "w1": _w((lambda *s: _rng.normal(s) * 0.05)(D, F) * (2.0 / D) ** 0.5),
            "w3": _w((lambda *s: _rng.normal(s) * 0.05)(D, F) * (2.0 / D) ** 0.5),
            "w2": _w((lambda *s: _rng.normal(s) * 0.05)(F, D) * (2.0 / F) ** 0.5),
        }
    _B_in = _B_setup()

    return {
        "A_x": _A_in["x"],
        "A_k_cache": _A_in["k_cache"],
        "A_v_cache": _A_in["v_cache"],
        "A_wq": _A_in["wq"],
        "A_wo": _A_in["wo"],
        "B_x": _B_in["x"],
        "B_w1": _B_in["w1"],
        "B_w3": _B_in["w3"],
        "B_w2": _B_in["w2"],
    }

def reference(A_x, A_k_cache, A_v_cache, A_wq, A_wo, B_x, B_w1, B_w3, B_w2):
    def _A_ref(x, k_cache, v_cache, wq, wo):
        B, Sq, D = x.shape
        Hq, Dh = 32, 192
        Hkv, Sk = k_cache.shape[1], k_cache.shape[2]
        W = min(4096, max(256, Sk // 4))
        rep = Hq // Hkv
        q = (lambda x, *d: x.transpose(*d))((x @ wq).reshape(B, Sq, Hq, Dh), 0, 2, 1, 3)
        k = jnp.repeat(k_cache[:, :, Sk - W:, :], rep, axis=1)
        v = jnp.repeat(v_cache[:, :, Sk - W:, :], rep, axis=1)
        scores = jnp.einsum("bhqd,bhkd->bhqk", q, k) * (Dh ** -0.5)
        p = _softmax(scores, axis=-1)
        o = jnp.einsum("bhqk,bhkd->bhqd", p, v)
        return (lambda x, *d: x.transpose(*d))(o, 0, 2, 1, 3).reshape(B, Sq, Hq * Dh) @ wo

    def _B_ref(x, w1, w3, w2):
        gate = jnp.einsum("bsd,df->bsf", x, w1)
        up = jnp.einsum("bsd,df->bsf", x, w3)
        h = _silu(gate) * up
        out = jnp.einsum("bsf,fd->bsd", h, w2)
        return out

    x = A_x
    h = x + _A_ref(_layernorm(x, axis=-1), A_k_cache, A_v_cache, A_wq, A_wo)
    h2 = h + _B_ref(_layernorm(h, axis=-1), B_w1, B_w3, B_w2)
    return h2
```

```python
import functools

import jax
import jax.numpy as jnp
import jax.experimental.pallas as pl
import jax.experimental.pallas.tpu as pltpu

_HQ = 32
_DH = 192
_EPS = 1e-5
_ROWS = 8
_NBUF = 4
_WQ_CHUNK = 128
_F_CHUNK = 512
_W2_CHUNK = 256


def _layernorm(x):
    m = jnp.mean(x, axis=-1, keepdims=True)
    c = x - m
    v = jnp.mean(c * c, axis=-1, keepdims=True)
    return c / jnp.sqrt(v + _EPS)


def _kernel(x_hbm, k_hbm, v_hbm, wq_hbm, wo_hbm, w1_hbm, w3_hbm, w2_hbm, o_ref,
            x_v, wq_v, wo_v, w1_v, w3_v, w2_v, kbuf, vbuf, q_v,
            sem_x, sem_wq, sem_k, sem_v, sem_wo, sem_w1, sem_w3, sem_w2,
            *, win_start, win):
    f32, bf16 = jnp.float32, jnp.bfloat16
    d_model = x_v.shape[-1]
    d_ff = w1_v.shape[-1]
    n_wq = d_model // _WQ_CHUNK
    n_f = d_ff // _F_CHUNK
    n_w2 = d_ff // _W2_CHUNK

    def x_copy():
        return pltpu.make_async_copy(x_hbm, x_v, sem_x.at[0])

    def wq_copy(c):
        rows = pl.ds(c * _WQ_CHUNK, _WQ_CHUNK)
        return pltpu.make_async_copy(wq_hbm.at[rows, :], wq_v.at[rows, :], sem_wq.at[c])

    def k_copy(h, slot):
        return pltpu.make_async_copy(
            k_hbm.at[0, h, :, pl.ds(win_start, win)], kbuf.at[slot], sem_k.at[slot])

    def v_copy(h, slot):
        return pltpu.make_async_copy(
            v_hbm.at[0, h, :, pl.ds(win_start, win)], vbuf.at[slot], sem_v.at[slot])

    def wo_copy(h, slot):
        return pltpu.make_async_copy(wo_hbm.at[h], wo_v.at[slot], sem_wo.at[slot])

    def w1_copy(c):
        cols = pl.ds(c * _F_CHUNK, _F_CHUNK)
        return pltpu.make_async_copy(w1_hbm.at[:, cols], w1_v.at[:, cols], sem_w1.at[c])

    def w3_copy(c):
        cols = pl.ds(c * _F_CHUNK, _F_CHUNK)
        return pltpu.make_async_copy(w3_hbm.at[:, cols], w3_v.at[:, cols], sem_w3.at[c])

    def w2_copy(c):
        rows = pl.ds(c * _W2_CHUNK, _W2_CHUNK)
        return pltpu.make_async_copy(w2_hbm.at[rows, :], w2_v.at[rows, :], sem_w2.at[c])

    def start_head(h, slot):
        k_copy(h, slot).start()
        v_copy(h, slot).start()
        wo_copy(h, slot).start()

    x_copy().start()
    for c in range(n_wq):
        wq_copy(c).start()
    for h in range(_NBUF):
        start_head(h, h)

    x_copy().wait()
    x = jnp.broadcast_to(x_v[...].astype(f32), (_ROWS, d_model))
    xn = _layernorm(x).astype(bf16)

    q = jnp.zeros((_ROWS, _HQ * _DH), f32)
    for c in range(n_wq):
        wq_copy(c).wait()
        q = q + jnp.dot(xn[:, c * _WQ_CHUNK:(c + 1) * _WQ_CHUNK],
                        wq_v[c * _WQ_CHUNK:(c + 1) * _WQ_CHUNK, :],
                        preferred_element_type=f32)
    for h in range(_HQ):
        q_v[h] = q[:, h * _DH:(h + 1) * _DH].astype(bf16)

    scale = _DH ** -0.5

    def head_step(h, acc):
        slot = h % _NBUF
        k_copy(h, slot).wait()
        s = jnp.dot(q_v[h], kbuf[slot], preferred_element_type=f32) * scale
        m = jnp.max(s, axis=-1, keepdims=True)
        p = jnp.exp(s - m)
        l = jnp.sum(p, axis=-1, keepdims=True)
        v_copy(h, slot).wait()
        o = jax.lax.dot_general(p.astype(bf16), vbuf[slot], (((1,), (1,)), ((), ())),
                                preferred_element_type=f32)
        o = (o / l).astype(bf16)
        wo_copy(h, slot).wait()
        acc = acc + jnp.dot(o, wo_v[slot], preferred_element_type=f32)

        @pl.when(h + _NBUF < _HQ)
        def _():
            start_head(h + _NBUF, slot)

        @pl.when(h + _NBUF == _HQ)
        def _():
            for c in range(n_f):
                w1_copy(c).start()
                w3_copy(c).start()
            for c in range(n_w2):
                w2_copy(c).start()

        return acc

    attn = jax.lax.fori_loop(0, _HQ, head_step, jnp.zeros((_ROWS, d_model), f32))

    hres = x + attn
    hn = _layernorm(hres).astype(bf16)
    acts = []
    for c in range(n_f):
        cols = slice(c * _F_CHUNK, (c + 1) * _F_CHUNK)
        w1_copy(c).wait()
        g = jnp.dot(hn, w1_v[:, cols], preferred_element_type=f32)
        w3_copy(c).wait()
        u = jnp.dot(hn, w3_v[:, cols], preferred_element_type=f32)
        acts.append((g * jax.nn.sigmoid(g) * u).astype(bf16))
    act = jnp.concatenate(acts, axis=-1)
    out = hres
    for c in range(n_w2):
        rows = slice(c * _W2_CHUNK, (c + 1) * _W2_CHUNK)
        w2_copy(c).wait()
        out = out + jnp.dot(act[:, rows], w2_v[rows, :], preferred_element_type=f32)
    o_ref[...] = out[0:1, :].astype(o_ref.dtype)


@jax.jit
def pallas_sequential_preLN__sliding_block_cached__glu_gated_swiglu__decode_kernel(
    A_x: jax.Array,
    A_k_cache: jax.Array,
    A_v_cache: jax.Array,
    A_wq: jax.Array,
    A_wo: jax.Array,
    B_x: jax.Array,
    B_w1: jax.Array,
    B_w3: jax.Array,
    B_w2: jax.Array,
):
    del B_x
    b, sq, d_model = A_x.shape
    hkv, sk = A_k_cache.shape[1], A_k_cache.shape[2]
    d_ff = B_w1.shape[1]
    assert b == 1 and sq == 1 and hkv == _HQ and A_k_cache.shape[3] == _DH
    win = min(4096, max(256, sk // 4))
    bf16 = jnp.bfloat16

    k_t = jnp.swapaxes(A_k_cache, 2, 3)
    v_t = jnp.swapaxes(A_v_cache, 2, 3)
    x2 = A_x.reshape(1, d_model)
    wo3 = A_wo.reshape(_HQ, _DH, d_model)

    any_spec = pl.BlockSpec(memory_space=pl.ANY)
    dma = pltpu.SemaphoreType.DMA
    out = pl.pallas_call(
        functools.partial(_kernel, win_start=sk - win, win=win),
        out_shape=jax.ShapeDtypeStruct((1, d_model), A_x.dtype),
        in_specs=[any_spec] * 8,
        out_specs=pl.BlockSpec(memory_space=pltpu.VMEM),
        scratch_shapes=[
            pltpu.VMEM((1, d_model), bf16),
            pltpu.VMEM((d_model, _HQ * _DH), bf16),
            pltpu.VMEM((_NBUF, _DH, d_model), bf16),
            pltpu.VMEM((d_model, d_ff), bf16),
            pltpu.VMEM((d_model, d_ff), bf16),
            pltpu.VMEM((d_ff, d_model), bf16),
            pltpu.VMEM((_NBUF, _DH, win), bf16),
            pltpu.VMEM((_NBUF, _DH, win), bf16),
            pltpu.VMEM((_HQ, _ROWS, _DH), bf16),
            dma((1,)),
            dma((d_model // _WQ_CHUNK,)),
            dma((_NBUF,)),
            dma((_NBUF,)),
            dma((_NBUF,)),
            dma((d_ff // _F_CHUNK,)),
            dma((d_ff // _F_CHUNK,)),
            dma((d_ff // _W2_CHUNK,)),
        ],
        compiler_params=pltpu.CompilerParams(vmem_limit_bytes=64 * 1024 * 1024),
    )(x2, k_t, v_t, A_wq, wo3, B_w1, B_w3, B_w2)
    return out.reshape(b, sq, d_model)
```

```python
import functools

import jax
import jax.numpy as jnp
import jax.experimental.pallas as pl
import jax.experimental.pallas.tpu as pltpu

_HQ = 32
_DH = 192
_EPS = 1e-5
_ROWS = 8
_SC = 512
_RH = 96
_PAIR = 2 * _DH
_RB = 16
_HI, _LO = 0, 1
UNROLL = False


def _layernorm(x):
    m = jnp.mean(x, axis=-1, keepdims=True)
    c = x - m
    v = jnp.mean(c * c, axis=-1, keepdims=True)
    return c / jnp.sqrt(v + _EPS)


def _kernel(x_hbm, k_hbm, v_hbm, wq_hbm, wo_hbm, w1_hbm, w3_hbm, w2_hbm, o_ref,
            x_v, xn_v, wq_v, wo_v, w1_v, w3_v, w2_v, kbuf, vbuf, q_v, s_v, m_v,
            sem_x, sem_wq, sem_k, sem_v, sem_wo, sem_f1, sem_f0,
            *, win_start, win):
    f32, bf16 = jnp.float32, jnp.bfloat16
    d_model = x_v.shape[-1]
    d_ff = w1_v.shape[-1]
    n_sl = win // _SC
    n_half = n_sl * (_DH // _RH)
    n_wq = d_model // _RB // 2
    n_wo = _DH // _RB
    assert n_half == 16 and n_wq == 20 and n_wo == 12
    scale = _DH ** -0.5
    mult = pl.multiple_of

    def loop(lo, hi, body, carry):
        if UNROLL:
            for i in range(lo, hi):
                carry = body(i, carry)
            return carry
        return jax.lax.fori_loop(lo, hi, body, carry)

    def ds(start, size, align):
        if isinstance(start, int):
            return pl.ds(start, size)
        return pl.ds(mult(start, align), size)

    def kv_copy(hbm, buf, sem, h, t):
        slot = h % 2
        rows = ds((t % 2) * _RH, _RH, _RH)
        c = (t // 2) * _SC
        return pltpu.make_async_copy(
            hbm.at[0, h, rows, ds(win_start + c, _SC, _SC)],
            buf.at[slot, rows, ds(c, _SC, _SC)], sem.at[slot])

    k_copy = functools.partial(kv_copy, k_hbm, kbuf, sem_k)
    v_copy = functools.partial(kv_copy, v_hbm, vbuf, sem_v)

    def wq_copy(pair, r0, nrows, align=_RB):
        rows = ds(r0, nrows, align)
        return pltpu.make_async_copy(
            wq_hbm.at[rows, ds(pair * _PAIR, _PAIR, 128)],
            wq_v.at[pair % 2, rows, :], sem_wq.at[pair % 2])

    def wo_copy(h, b):
        rows = ds(b * _RB, _RB, _RB)
        return pltpu.make_async_copy(wo_hbm.at[h, rows, :], wo_v.at[h % 2, rows, :],
                                     sem_wo.at[h % 2])

    def wait_all(ref, sem):
        pltpu.make_async_copy(ref, ref, sem).wait()

    n_slab = d_ff // _PAIR
    def up_copy(hbm, buf, slab, r0, nrows, sem, align=_RB):
        rows = ds(r0, nrows, align)
        cols = pl.ds(slab * _PAIR, _PAIR)
        return pltpu.make_async_copy(hbm.at[rows, cols], buf.at[rows, cols], sem)

    def w2_copy(r0, nrows, sem):
        rows = pl.ds(r0, nrows)
        return pltpu.make_async_copy(w2_hbm.at[rows, :], w2_v.at[rows, :], sem)

    w2_hi_rows = 256
    ffn_lo = []
    for slab in range(1, n_slab):
        for r in range(0, d_model, 128):
            ffn_lo.append(("w1", slab, r, 128))
    for slab in range(0, n_slab - 1):
        for r in range(0, d_model, 128):
            ffn_lo.append(("w3", slab, r, 128))
    for r in range(w2_hi_rows, d_ff, 64):
        ffn_lo.append(("w2", 0, r, 64))

    def ffn_lo_copy(i):
        kind, slab, r, n = ffn_lo[i]
        sem = sem_f1.at[i]
        if kind == "w1":
            return up_copy(w1_hbm, w1_v, slab, r, n, sem)
        if kind == "w3":
            return up_copy(w3_hbm, w3_v, slab, r, n, sem)
        return w2_copy(r, n, sem)

    ffn_hi = [("w3", r) for r in range(0, d_model, 32)] + \
             [("w2", r) for r in range(0, w2_hi_rows, _RB)]

    def ffn_hi_copy(i):
        kind, r = ffn_hi[i]
        if kind == "w3":
            return up_copy(w3_hbm, w3_v, n_slab - 1, r, 32, sem_f0.at[1])
        return w2_copy(r, _RB, sem_f0.at[2])

    def start_wq_piece(j, b):
        r0 = ((j % 2) * n_wq + b) * _RB

        @pl.when(j < _HQ - 2)
        def _():
            wq_copy(j // 2 + 1, r0, _RB).start(priority=_HI)

        @pl.when(j >= _HQ - 2)
        def _():
            up_copy(w1_hbm, w1_v, 0, r0, _RB, sem_f0.at[0]).start(priority=_HI)

    def qk_slice(h, i, mx):
        cols = ds(i * _SC, _SC, _SC)
        s = jnp.dot(q_v[h % 2], kbuf[h % 2, :, cols], preferred_element_type=f32) * scale
        s_v[:, cols] = s
        for c in range(_SC // 128):
            mx = jnp.maximum(mx, s[:, c * 128:(c + 1) * 128])
        return mx

    def pv_slice(h, i, carry):
        acc, den = carry
        cols = ds(i * _SC, _SC, _SC)
        p = jnp.exp(s_v[:, cols] - m_v[:, 0:1])
        for c in range(_SC // 128):
            den = den + p[:, c * 128:(c + 1) * 128]
        acc = acc + jax.lax.dot_general(
            p.astype(bf16), vbuf[h % 2, :, cols], (((1,), (1,)), ((), ())),
            preferred_element_type=f32)
        return acc, den

    def pv_init():
        return jnp.zeros((_ROWS, _DH), f32), jnp.zeros((_ROWS, 128), f32)

    def out_proj(h, acc, den):
        o = (acc / jnp.sum(den, axis=-1, keepdims=True)).astype(bf16)
        wait_all(wo_v.at[h % 2], sem_wo.at[h % 2])
        return jnp.dot(o, wo_v[h % 2], preferred_element_type=f32)

    def q_proj(pair):
        wait_all(wq_v.at[pair % 2], sem_wq.at[pair % 2])
        q = jnp.dot(xn_v[...], wq_v[pair % 2], preferred_element_type=f32).astype(bf16)
        q_v[0] = q[:, :_DH]
        q_v[1] = q[:, _DH:]

    x_copy = pltpu.make_async_copy(x_hbm, x_v, sem_x.at[0])
    x_copy.start(priority=_HI)
    for r in range(0, d_model, 128):
        wq_copy(0, r, 128).start(priority=_LO)
    for t in range(n_half):
        k_copy(0, t).start(priority=_LO)
    x_copy.wait()
    x = jnp.broadcast_to(x_v[...].astype(f32), (_ROWS, d_model))
    xn_v[...] = _layernorm(x).astype(bf16)

    def phase(j, attn):
        def tick_a(t):
            k_copy(j, t).wait()
            start_wq_piece(j, t)
            v_copy(j, t).start(priority=_LO)

        def a_pv(t, carry):
            tick_a(t)
            return pv_slice(j + 1, t, carry)

        def a_idle(t, carry):
            tick_a(t)
            return carry

        def with_prev(attn):
            acc, den = loop(0, n_sl, a_pv, pv_init())
            tick_a(n_sl)
            return attn + out_proj(j + 1, acc, den)

        def without_prev(attn):
            loop(0, n_sl + 1, a_idle, 0)
            return attn

        attn = jax.lax.cond(j > 0, with_prev, without_prev, attn)
        tick_a(n_sl + 1)

        @pl.when(j % 2 == 0)
        def _():
            q_proj(j // 2)

        loop(n_sl + 2, n_half, a_idle, 0)

        def start_next_lo(t):
            @pl.when(j + 1 < _HQ)
            def _():
                k_copy(j + 1, t).start(priority=_LO)

        def b_qk(t, mx):
            v_copy(j, t).wait()
            wo_copy(j, t).start(priority=_HI)
            start_next_lo(t)
            return qk_slice(j, t, mx)

        def b_wo(t, c):
            v_copy(j, t).wait()
            wo_copy(j, t).start(priority=_HI)
            start_next_lo(t)
            return c

        def b_wq(t, c):
            v_copy(j, t).wait()
            start_wq_piece(j, t + (n_half - n_wo))
            start_next_lo(t)
            return c

        @pl.when(j + 1 == _HQ)
        def _():
            for i in range(n_half):
                ffn_lo_copy(i).start(priority=_LO)

        mx = loop(0, n_sl, b_qk, jnp.full((_ROWS, 128), -jnp.inf, f32))
        m_v[...] = jnp.broadcast_to(jnp.max(mx, axis=-1, keepdims=True), (_ROWS, 128))
        loop(n_sl, n_wo, b_wo, 0)
        loop(n_wo, n_half, b_wq, 0)
        return attn

    attn = jax.lax.fori_loop(0, _HQ, phase, jnp.zeros((_ROWS, d_model), f32))

    n_lo = len(ffn_lo)

    def tick_f(i):
        ffn_lo_copy(i).wait()
        if i < len(ffn_hi):
            ffn_hi_copy(i).start(priority=_HI)
        if i + n_half < n_lo:
            ffn_lo_copy(i + n_half).start(priority=_LO)

    last = _HQ - 1
    carry = pv_init()
    for i in range(n_sl):
        tick_f(i)
        carry = pv_slice(last, i, carry)
    tick_f(n_sl)
    hres = x + attn + out_proj(last, *carry)
    hn = _layernorm(hres).astype(bf16)

    def slab_dot(buf, slab):
        return jnp.dot(hn, buf[:, slab * _PAIR:(slab + 1) * _PAIR], preferred_element_type=f32)

    per_slab = d_model // 128
    gates, ups = {}, {}
    tick_f(9)
    wait_all(w1_v.at[:, pl.ds(0, _PAIR)], sem_f0.at[0])
    gates[0] = slab_dot(w1_v, 0)
    tick_f(10)
    gates[1] = slab_dot(w1_v, 1)
    tick_f(11)
    gates[2] = slab_dot(w1_v, 2)
    for i in range(12, 15):
        tick_f(i)
    gates[3] = slab_dot(w1_v, 3)
    for i in range(15, 20):
        tick_f(i)
    ups[0] = slab_dot(w3_v, 0)
    for i in range(20, 25):
        tick_f(i)
    ups[1] = slab_dot(w3_v, 1)
    for i in range(25, 28):
        tick_f(i)
    wait_all(w3_v.at[:, pl.ds((n_slab - 1) * _PAIR, _PAIR)], sem_f0.at[1])
    ups[3] = slab_dot(w3_v, 3)
    for i in range(28, 30):
        tick_f(i)
    ups[2] = slab_dot(w3_v, 2)
    act = jnp.concatenate(
        [(gates[s] * jax.nn.sigmoid(gates[s]) * ups[s]).astype(bf16) for s in range(n_slab)],
        axis=-1)

    def down(r0, n):
        return jnp.dot(act[:, r0:r0 + n], w2_v[r0:r0 + n, :], preferred_element_type=f32)

    out = hres
    first_w2 = 30
    for i in range(first_w2, n_lo):
        tick_f(i)
        k = i - first_w2
        if k % 2 == 1:
            out = out + down(w2_hi_rows + (k - 1) * 64, 128)
        if i == n_lo - 5:
            wait_all(w2_v.at[pl.ds(0, w2_hi_rows), :], sem_f0.at[2])
            out = out + down(0, w2_hi_rows)
    o_ref[...] = out[0:1, :].astype(o_ref.dtype)


@jax.jit
def pallas_sequential_preLN__sliding_block_cached__glu_gated_swiglu__decode_kernel(
    A_x: jax.Array,
    A_k_cache: jax.Array,
    A_v_cache: jax.Array,
    A_wq: jax.Array,
    A_wo: jax.Array,
    B_x: jax.Array,
    B_w1: jax.Array,
    B_w3: jax.Array,
    B_w2: jax.Array,
):
    del B_x
    b, sq, d_model = A_x.shape
    hkv, sk = A_k_cache.shape[1], A_k_cache.shape[2]
    d_ff = B_w1.shape[1]
    assert b == 1 and sq == 1 and hkv == _HQ and A_k_cache.shape[3] == _DH
    win = min(4096, max(256, sk // 4))
    bf16, f32 = jnp.bfloat16, jnp.float32

    k_t = jnp.swapaxes(A_k_cache, 2, 3)
    v_t = jnp.swapaxes(A_v_cache, 2, 3)
    x2 = A_x.reshape(1, d_model)
    wo3 = A_wo.reshape(_HQ, _DH, d_model)

    any_spec = pl.BlockSpec(memory_space=pl.ANY)
    dma = pltpu.SemaphoreType.DMA
    out = pl.pallas_call(
        functools.partial(_kernel, win_start=sk - win, win=win),
        out_shape=jax.ShapeDtypeStruct((1, d_model), A_x.dtype),
        in_specs=[any_spec] * 8,
        out_specs=pl.BlockSpec(memory_space=pltpu.VMEM),
        scratch_shapes=[
            pltpu.VMEM((1, d_model), bf16),
            pltpu.VMEM((_ROWS, d_model), bf16),
            pltpu.VMEM((2, d_model, _PAIR), bf16),
            pltpu.VMEM((2, _DH, d_model), bf16),
            pltpu.VMEM((d_model, d_ff), bf16),
            pltpu.VMEM((d_model, d_ff), bf16),
            pltpu.VMEM((d_ff, d_model), bf16),
            pltpu.VMEM((2, _DH, win), bf16),
            pltpu.VMEM((2, _DH, win), bf16),
            pltpu.VMEM((2, _ROWS, _DH), bf16),
            pltpu.VMEM((_ROWS, win), f32),
            pltpu.VMEM((_ROWS, 128), f32),
            dma((1,)), dma((2,)), dma((2,)), dma((2,)), dma((2,)),
            dma((50,)), dma((3,)),
        ],
        compiler_params=pltpu.CompilerParams(vmem_limit_bytes=48 * 1024 * 1024),
    )(x2, k_t, v_t, A_wq, wo3, B_w1, B_w3, B_w2)
    return out.reshape(b, sq, d_model)
```

```python
import functools

import jax
import jax.numpy as jnp
import jax.experimental.pallas as pl
import jax.experimental.pallas.tpu as pltpu

_HQ = 32
_DH = 192
_EPS = 1e-5
_ROWS = 8
_SC = 512
_KV_R, _KV_C = 48, 1024
_PAIR = 2 * _DH
_RB = 16
_HI, _LO = 0, 1
UNROLL = False


def _layernorm(x):
    m = jnp.mean(x, axis=-1, keepdims=True)
    c = x - m
    v = jnp.mean(c * c, axis=-1, keepdims=True)
    return c / jnp.sqrt(v + _EPS)


def _kernel(x_hbm, k_hbm, v_hbm, wq_hbm, wo_hbm, w1_hbm, w3_hbm, w2_hbm, o_ref,
            x_v, xn_v, wq_v, wo_v, w1_v, w3_v, w2_v, kbuf, vbuf, q_v, s_v, m_v,
            sem_x, sem_wq, sem_k, sem_v, sem_wo, sem_f1, sem_f0,
            *, win_start, win):
    f32, bf16 = jnp.float32, jnp.bfloat16
    d_model = x_v.shape[-1]
    d_ff = w1_v.shape[-1]
    n_sl = win // _SC
    n_rb = _DH // _KV_R
    n_half = n_rb * (win // _KV_C)
    n_wq = d_model // _RB // 2
    n_wo = _DH // _RB
    assert n_half == 16 and n_wq == 20 and n_wo == 12
    scale = _DH ** -0.5
    mult = pl.multiple_of

    def loop(lo, hi, body, carry):
        if UNROLL:
            for i in range(lo, hi):
                carry = body(i, carry)
            return carry
        return jax.lax.fori_loop(lo, hi, body, carry)

    def ds(start, size, align):
        if isinstance(start, int):
            return pl.ds(start, size)
        return pl.ds(mult(start, align), size)

    def kv_copy(hbm, buf, sem, h, t):
        slot = h % 2
        rows = ds((t % n_rb) * _KV_R, _KV_R, _RB)
        c = (t // n_rb) * _KV_C
        return pltpu.make_async_copy(
            hbm.at[0, h, rows, ds(win_start + c, _KV_C, _KV_C)],
            buf.at[slot, rows, ds(c, _KV_C, _KV_C)], sem.at[slot])

    k_copy = functools.partial(kv_copy, k_hbm, kbuf, sem_k)
    v_copy = functools.partial(kv_copy, v_hbm, vbuf, sem_v)

    def wq_copy(pair, r0, nrows, align=_RB):
        rows = ds(r0, nrows, align)
        return pltpu.make_async_copy(
            wq_hbm.at[rows, ds(pair * _PAIR, _PAIR, 128)],
            wq_v.at[pair % 2, rows, :], sem_wq.at[pair % 2])

    def wo_copy(h, b):
        rows = ds(b * _RB, _RB, _RB)
        return pltpu.make_async_copy(wo_hbm.at[h, rows, :], wo_v.at[h % 2, rows, :],
                                     sem_wo.at[h % 2])

    def wait_all(ref, sem):
        pltpu.make_async_copy(ref, ref, sem).wait()

    n_slab = d_ff // _PAIR
    def up_copy(hbm, buf, slab, r0, nrows, sem, align=_RB):
        rows = ds(r0, nrows, align)
        cols = pl.ds(slab * _PAIR, _PAIR)
        return pltpu.make_async_copy(hbm.at[rows, cols], buf.at[rows, cols], sem)

    def w2_copy(r0, nrows, sem):
        rows = pl.ds(r0, nrows)
        return pltpu.make_async_copy(w2_hbm.at[rows, :], w2_v.at[rows, :], sem)

    w2_hi_rows = 256
    ffn_lo = []
    for slab in range(1, n_slab):
        for r in range(0, d_model, 128):
            ffn_lo.append(("w1", slab, r, 128))
    for slab in range(0, n_slab - 1):
        for r in range(0, d_model, 128):
            ffn_lo.append(("w3", slab, r, 128))
    for r in range(w2_hi_rows, d_ff, 64):
        ffn_lo.append(("w2", 0, r, 64))

    def ffn_lo_copy(i):
        kind, slab, r, n = ffn_lo[i]
        sem = sem_f1.at[i]
        if kind == "w1":
            return up_copy(w1_hbm, w1_v, slab, r, n, sem)
        if kind == "w3":
            return up_copy(w3_hbm, w3_v, slab, r, n, sem)
        return w2_copy(r, n, sem)

    ffn_hi = [("w3", r) for r in range(0, d_model, 32)] + \
             [("w2", r) for r in range(0, w2_hi_rows, _RB)]

    def ffn_hi_copy(i):
        kind, r = ffn_hi[i]
        if kind == "w3":
            return up_copy(w3_hbm, w3_v, n_slab - 1, r, 32, sem_f0.at[1])
        return w2_copy(r, _RB, sem_f0.at[2])

    def start_wq_piece(j, b):
        r0 = ((j % 2) * n_wq + b) * _RB

        @pl.when(j < _HQ - 2)
        def _():
            wq_copy(j // 2 + 1, r0, _RB).start(priority=_HI)

        @pl.when(j >= _HQ - 2)
        def _():
            up_copy(w1_hbm, w1_v, 0, r0, _RB, sem_f0.at[0]).start(priority=_HI)

    def qk_slice(h, i, mx):
        cols = ds(i * _SC, _SC, _SC)
        s = jnp.dot(q_v[h % 2], kbuf[h % 2, :, cols], preferred_element_type=f32) * scale
        s_v[:, cols] = s
        for c in range(_SC // 128):
            mx = jnp.maximum(mx, s[:, c * 128:(c + 1) * 128])
        return mx

    def pv_slice(h, i, carry):
        acc, den = carry
        cols = ds(i * _SC, _SC, _SC)
        p = jnp.exp(s_v[:, cols] - m_v[:, 0:1])
        for c in range(_SC // 128):
            den = den + p[:, c * 128:(c + 1) * 128]
        acc = acc + jax.lax.dot_general(
            p.astype(bf16), vbuf[h % 2, :, cols], (((1,), (1,)), ((), ())),
            preferred_element_type=f32)
        return acc, den

    def pv_init():
        return jnp.zeros((_ROWS, _DH), f32), jnp.zeros((_ROWS, 128), f32)

    def out_proj(h, acc, den):
        o = (acc / jnp.sum(den, axis=-1, keepdims=True)).astype(bf16)
        wait_all(wo_v.at[h % 2], sem_wo.at[h % 2])
        return jnp.dot(o, wo_v[h % 2], preferred_element_type=f32)

    def q_proj(pair):
        wait_all(wq_v.at[pair % 2], sem_wq.at[pair % 2])
        q = jnp.dot(xn_v[...], wq_v[pair % 2], preferred_element_type=f32).astype(bf16)
        q_v[0] = q[:, :_DH]
        q_v[1] = q[:, _DH:]

    x_copy = pltpu.make_async_copy(x_hbm, x_v, sem_x.at[0])
    x_copy.start(priority=_HI)
    for r in range(0, d_model, 128):
        wq_copy(0, r, 128).start(priority=_LO)
    for t in range(n_half):
        k_copy(0, t).start(priority=_LO)
    x_copy.wait()
    x = jnp.broadcast_to(x_v[...].astype(f32), (_ROWS, d_model))
    xn_v[...] = _layernorm(x).astype(bf16)

    def phase(j, attn):
        def tick_a(t):
            k_copy(j, t).wait()
            start_wq_piece(j, t)
            v_copy(j, t).start(priority=_LO)

        def a_pv(t, carry):
            tick_a(t)
            return pv_slice(j + 1, t, carry)

        def a_idle(t, carry):
            tick_a(t)
            return carry

        def with_prev(attn):
            acc, den = loop(0, n_sl, a_pv, pv_init())
            tick_a(n_sl)
            return attn + out_proj(j + 1, acc, den)

        def without_prev(attn):
            loop(0, n_sl + 1, a_idle, 0)
            return attn

        attn = jax.lax.cond(j > 0, with_prev, without_prev, attn)
        tick_a(n_sl + 1)

        @pl.when(j % 2 == 0)
        def _():
            q_proj(j // 2)

        loop(n_sl + 2, n_half, a_idle, 0)

        def start_next_lo(t):
            @pl.when(j + 1 < _HQ)
            def _():
                k_copy(j + 1, t).start(priority=_LO)

        def b_qk(t, mx):
            v_copy(j, t).wait()
            wo_copy(j, t).start(priority=_HI)
            start_next_lo(t)
            return qk_slice(j, t, mx)

        def b_wo(t, c):
            v_copy(j, t).wait()
            wo_copy(j, t).start(priority=_HI)
            start_next_lo(t)
            return c

        def b_wq(t, c):
            v_copy(j, t).wait()
            start_wq_piece(j, t + (n_half - n_wo))
            start_next_lo(t)
            return c

        @pl.when(j + 1 == _HQ)
        def _():
            for i in range(n_half):
                ffn_lo_copy(i).start(priority=_LO)

        mx = loop(0, n_sl, b_qk, jnp.full((_ROWS, 128), -jnp.inf, f32))
        m_v[...] = jnp.broadcast_to(jnp.max(mx, axis=-1, keepdims=True), (_ROWS, 128))
        loop(n_sl, n_wo, b_wo, 0)
        loop(n_wo, n_half, b_wq, 0)
        return attn

    attn = jax.lax.fori_loop(0, _HQ, phase, jnp.zeros((_ROWS, d_model), f32))

    n_lo = len(ffn_lo)

    def tick_f(i):
        ffn_lo_copy(i).wait()
        if i < len(ffn_hi):
            ffn_hi_copy(i).start(priority=_HI)
        if i + n_half < n_lo:
            ffn_lo_copy(i + n_half).start(priority=_LO)

    last = _HQ - 1
    carry = pv_init()
    for i in range(n_sl):
        tick_f(i)
        carry = pv_slice(last, i, carry)
    tick_f(n_sl)
    hres = x + attn + out_proj(last, *carry)
    hn = _layernorm(hres).astype(bf16)

    def slab_dot(buf, slab):
        return jnp.dot(hn, buf[:, slab * _PAIR:(slab + 1) * _PAIR], preferred_element_type=f32)

    per_slab = d_model // 128
    gates, ups = {}, {}
    tick_f(9)
    wait_all(w1_v.at[:, pl.ds(0, _PAIR)], sem_f0.at[0])
    gates[0] = slab_dot(w1_v, 0)
    tick_f(10)
    gates[1] = slab_dot(w1_v, 1)
    tick_f(11)
    gates[2] = slab_dot(w1_v, 2)
    for i in range(12, 15):
        tick_f(i)
    gates[3] = slab_dot(w1_v, 3)
    for i in range(15, 20):
        tick_f(i)
    ups[0] = slab_dot(w3_v, 0)
    for i in range(20, 25):
        tick_f(i)
    ups[1] = slab_dot(w3_v, 1)
    for i in range(25, 28):
        tick_f(i)
    wait_all(w3_v.at[:, pl.ds((n_slab - 1) * _PAIR, _PAIR)], sem_f0.at[1])
    ups[3] = slab_dot(w3_v, 3)
    for i in range(28, 30):
        tick_f(i)
    ups[2] = slab_dot(w3_v, 2)
    act = jnp.concatenate(
        [(gates[s] * jax.nn.sigmoid(gates[s]) * ups[s]).astype(bf16) for s in range(n_slab)],
        axis=-1)

    def down(r0, n):
        return jnp.dot(act[:, r0:r0 + n], w2_v[r0:r0 + n, :], preferred_element_type=f32)

    out = hres
    first_w2 = 30
    for i in range(first_w2, n_lo):
        tick_f(i)
        k = i - first_w2
        if k % 2 == 1:
            out = out + down(w2_hi_rows + (k - 1) * 64, 128)
        if i == n_lo - 5:
            wait_all(w2_v.at[pl.ds(0, w2_hi_rows), :], sem_f0.at[2])
            out = out + down(0, w2_hi_rows)
    o_ref[...] = out[0:1, :].astype(o_ref.dtype)


@jax.jit
def pallas_sequential_preLN__sliding_block_cached__glu_gated_swiglu__decode_kernel(
    A_x: jax.Array,
    A_k_cache: jax.Array,
    A_v_cache: jax.Array,
    A_wq: jax.Array,
    A_wo: jax.Array,
    B_x: jax.Array,
    B_w1: jax.Array,
    B_w3: jax.Array,
    B_w2: jax.Array,
):
    del B_x
    b, sq, d_model = A_x.shape
    hkv, sk = A_k_cache.shape[1], A_k_cache.shape[2]
    d_ff = B_w1.shape[1]
    assert b == 1 and sq == 1 and hkv == _HQ and A_k_cache.shape[3] == _DH
    win = min(4096, max(256, sk // 4))
    bf16, f32 = jnp.bfloat16, jnp.float32

    k_t = jnp.swapaxes(A_k_cache, 2, 3)
    v_t = jnp.swapaxes(A_v_cache, 2, 3)
    x2 = A_x.reshape(1, d_model)
    wo3 = A_wo.reshape(_HQ, _DH, d_model)

    any_spec = pl.BlockSpec(memory_space=pl.ANY)
    dma = pltpu.SemaphoreType.DMA
    out = pl.pallas_call(
        functools.partial(_kernel, win_start=sk - win, win=win),
        out_shape=jax.ShapeDtypeStruct((1, d_model), A_x.dtype),
        in_specs=[any_spec] * 8,
        out_specs=pl.BlockSpec(memory_space=pltpu.VMEM),
        scratch_shapes=[
            pltpu.VMEM((1, d_model), bf16),
            pltpu.VMEM((_ROWS, d_model), bf16),
            pltpu.VMEM((2, d_model, _PAIR), bf16),
            pltpu.VMEM((2, _DH, d_model), bf16),
            pltpu.VMEM((d_model, d_ff), bf16),
            pltpu.VMEM((d_model, d_ff), bf16),
            pltpu.VMEM((d_ff, d_model), bf16),
            pltpu.VMEM((2, _DH, win), bf16),
            pltpu.VMEM((2, _DH, win), bf16),
            pltpu.VMEM((2, _ROWS, _DH), bf16),
            pltpu.VMEM((_ROWS, win), f32),
            pltpu.VMEM((_ROWS, 128), f32),
            dma((1,)), dma((2,)), dma((2,)), dma((2,)), dma((2,)),
            dma((50,)), dma((3,)),
        ],
        compiler_params=pltpu.CompilerParams(vmem_limit_bytes=48 * 1024 * 1024),
    )(x2, k_t, v_t, A_wq, wo3, B_w1, B_w3, B_w2)
    return out.reshape(b, sq, d_model)
```

```python
import functools

import jax
import jax.numpy as jnp
import jax.experimental.pallas as pl
import jax.experimental.pallas.tpu as pltpu

_HQ = 32
_DH = 192
_EPS = 1e-5
_ROWS = 8
_KV_R, _KV_C = 48, 1024
_PAIR = 2 * _DH
_RB = 16
_HI, _LO = 0, 1
_W2_HI = 256

PV_SL = 8
QK_SL = 8
QK_TICKS = 8
PV_POS = 0
BOUNDS = True
SCOPES = False


def _layernorm(x):
    m = jnp.mean(x, axis=-1, keepdims=True)
    c = x - m
    v = jnp.mean(c * c, axis=-1, keepdims=True)
    return c / jnp.sqrt(v + _EPS)


def _kernel(x_hbm, k_hbm, v_hbm, wq_hbm, wo_hbm, w1_hbm, w3_hbm, w2_hbm, o_ref,
            x_v, xn_v, wq_v, wo_v, w1_v, w3_v, w2_v, kbuf, vbuf, q_v, s_v, m_v, av_v, attn_v,
            sem_x, sem_wq, sem_k, sem_v, sem_wo, sem_f1, sem_f0,
            *, win_start, win):
    f32, bf16 = jnp.float32, jnp.bfloat16
    d_model = x_v.shape[-1]
    d_ff = w1_v.shape[-1]
    n_half = (_DH // _KV_R) * (win // _KV_C)
    n_wq = d_model // _RB // 2
    n_wo = _DH // _RB
    assert _DH // _KV_R == 4 and n_half == 16 and n_wq + n_wo == 2 * n_half
    assert d_ff == 4 * _PAIR and d_model % 128 == 0
    scale = _DH ** -0.5

    def ds(start, size, align):
        if isinstance(start, int):
            return pl.ds(start, size)
        return pl.ds(pl.multiple_of(start, align), size)

    def kv_copy(hbm, buf, sem, h, slot, t):
        rows = ds((t & 3) * _KV_R, _KV_R, _RB)
        c = (t >> 2) * _KV_C
        return pltpu.make_async_copy(
            hbm.at[0, h, rows, ds(win_start + c, _KV_C, _KV_C)],
            buf.at[slot, rows, ds(c, _KV_C, _KV_C)], sem.at[slot])

    k_copy = functools.partial(kv_copy, k_hbm, kbuf, sem_k)
    v_copy = functools.partial(kv_copy, v_hbm, vbuf, sem_v)

    def wq_copy(pair, slot, r0, nrows):
        rows = ds(r0, nrows, _RB)
        return pltpu.make_async_copy(
            wq_hbm.at[rows, ds(pair * _PAIR, _PAIR, 128)],
            wq_v.at[slot, rows, :], sem_wq.at[slot])

    def wo_copy(h, slot, b):
        rows = ds(b * _RB, _RB, _RB)
        return pltpu.make_async_copy(wo_hbm.at[h, rows, :], wo_v.at[slot, rows, :],
                                     sem_wo.at[slot])

    def block_copy(hbm, buf, r0, nrows, c0, ncols, sem):
        rows, cols = ds(r0, nrows, _RB), ds(c0, ncols, 128)
        return pltpu.make_async_copy(hbm.at[rows, cols], buf.at[rows, cols], sem)

    def wait_all(ref, sem):
        pltpu.make_async_copy(ref, ref, sem).wait()

    w1_hi = 2 * n_wq * _RB // 4
    w3_lo = d_model - w1_hi
    ffn_lo = ([(w1_hbm, w1_v, r, 32, d_ff) for r in range(w1_hi, d_model, 32)]
              + [(w3_hbm, w3_v, r, 32, d_ff) for r in range(0, w3_lo, 32)]
              + [(w2_hbm, w2_v, r, 64, d_model) for r in range(_W2_HI, d_ff, 64)])
    ffn_hi = ([(w3_hbm, w3_v, r, c, d_ff // 2, 1)
               for r in range(w3_lo, d_model, _RB) for c in (0, d_ff // 2)]
              + [(w2_hbm, w2_v, r, 0, d_model, 2) for r in range(0, _W2_HI, _RB)])

    def ffn_lo_copy(i):
        hbm, buf, r, n, ncols = ffn_lo[i]
        return block_copy(hbm, buf, r, n, 0, ncols, sem_f1.at[i])

    def ffn_hi_copy(i):
        hbm, buf, r, c, ncols, s = ffn_hi[i]
        return block_copy(hbm, buf, r, _RB, c, ncols, sem_f0.at[s])

    def qk_slice(slot, i, mx):
        w = win // QK_SL
        cols = ds(i * w, w, w)
        s = jnp.dot(q_v[slot], kbuf[slot, :, cols], preferred_element_type=f32) * scale
        s_v[:, cols] = s
        for c in range(w // 128):
            mx = jnp.maximum(mx, s[:, c * 128:(c + 1) * 128])
        return mx

    def pv_slice(slot, i, carry):
        w = win // PV_SL
        acc, den = carry
        cols = ds(i * w, w, w)
        m = m_v[...]
        p = jnp.exp(s_v[:, cols] - jnp.concatenate([m] * (w // 128), axis=-1))
        for c in range(w // 128):
            den = den + p[:, c * 128:(c + 1) * 128]
        acc = acc + jax.lax.dot_general(
            p.astype(bf16), vbuf[slot, :, cols], (((1,), (1,)), ((), ())),
            preferred_element_type=f32)
        return acc, den

    def pv_init():
        return jnp.zeros((_ROWS, _DH), f32), jnp.zeros((_ROWS, 128), f32)

    def pv_finish(acc, den):
        return (acc / jnp.sum(den, axis=-1, keepdims=True)).astype(bf16)

    def out_proj(slot, o):
        wait_all(wo_v.at[slot], sem_wo.at[slot])
        return jnp.dot(o, wo_v[slot], preferred_element_type=f32)

    def q_proj(slot):
        wait_all(wq_v.at[slot], sem_wq.at[slot])
        q = jnp.dot(xn_v[...], wq_v[slot], preferred_element_type=f32).astype(bf16)
        q_v[0] = q[:, :_DH]
        q_v[1] = q[:, _DH:]

    x_copy = pltpu.make_async_copy(x_hbm, x_v, sem_x.at[0])
    x_copy.start(priority=_HI)
    for r in range(0, d_model, 128):
        wq_copy(0, 0, r, 128).start(priority=_LO)
    for t in range(n_half):
        k_copy(0, 0, t).start(priority=_LO)
    x_copy.wait()
    x = jnp.broadcast_to(x_v[...].astype(f32), (_ROWS, d_model))
    xn_v[...] = _layernorm(x).astype(bf16)
    attn_v[...] = x

    def phase(j, _):
        slot = j & 1
        prev = 1 - slot
        pair = (j >> 1) + 1
        pslot = pair & 1
        blk0 = slot * n_wq

        def start_wq_piece(b):
            blk = blk0 + b

            @pl.when(j < _HQ - 2)
            def _():
                wq_copy(pair, pslot, blk * _RB, _RB).start(priority=_HI)

            @pl.when(j >= _HQ - 2)
            def _():
                block_copy(w1_hbm, w1_v, (blk >> 2) * _RB, _RB, (blk & 3) * _PAIR, _PAIR,
                           sem_f0.at[0]).start(priority=_HI)

        def tick_a(t):
            k_copy(j, slot, t).wait()
            start_wq_piece(t)
            v_copy(j, slot, t).start(priority=_LO)

        g = n_half // PV_SL

        def a_pv(i, carry):
            for u in range(g):
                tick_a(i * g + u)
                if u == PV_POS:
                    carry = pv_slice(prev, i, carry)
            return carry

        def a_idle(t, c):
            tick_a(t)
            return c

        @pl.when(j > 0)
        def _():
            av_v[...] = pv_finish(*jax.lax.fori_loop(0, PV_SL, a_pv, pv_init()))

        @pl.when(j == 0)
        def _():
            jax.lax.fori_loop(0, n_half, a_idle, 0)
            q_proj(0)

        @pl.when(j + 1 == _HQ)
        def _():
            for i in range(n_half):
                ffn_lo_copy(i).start(priority=_LO)

        n_wq_b = n_wq - n_half

        def tick_b(t):
            v_copy(j, slot, t).wait()
            if isinstance(t, int):
                if t < n_wq_b:
                    start_wq_piece(n_half + t)
                else:
                    wo_copy(j, slot, t - n_wq_b).start(priority=_HI)
            else:
                @pl.when(t < n_wq_b)
                def _():
                    start_wq_piece(n_half + t)

                @pl.when(t >= n_wq_b)
                def _():
                    wo_copy(j, slot, t - n_wq_b).start(priority=_HI)

            @pl.when(j + 1 < _HQ)
            def _():
                k_copy(j + 1, prev, t).start(priority=_LO)

        gq = QK_TICKS // QK_SL

        def b_qk(i, mx):
            for u in range(gq):
                tick_b(i * gq + u)
                if u == 0:
                    mx = qk_slice(slot, i, mx)
            return mx

        def b_idle(t, c):
            tick_b(t)
            return c

        mx = jax.lax.fori_loop(0, QK_SL, b_qk, jnp.full((_ROWS, 128), -jnp.inf, f32))
        m_v[...] = jnp.broadcast_to(jnp.max(mx, axis=-1, keepdims=True), (_ROWS, 128))
        t_out = max(QK_TICKS, n_half - 4)
        t_out = min(t_out, n_half - 2)
        if QK_TICKS < n_half - 2:
            jax.lax.fori_loop(QK_TICKS, t_out, b_idle, 0)
        rest = list(range(max(t_out, QK_TICKS), n_half))

        def do_out():
            @pl.when(j > 0)
            def _():
                attn_v[...] += out_proj(prev, av_v[...])

        def do_q():
            @pl.when(jnp.logical_and(slot == 1, j + 1 < _HQ))
            def _():
                q_proj(pslot)

        todo = [do_out, do_q]
        for n, t in enumerate(rest):
            tick_b(t)
            if n % 2 == 0 and todo:
                todo.pop(0)()
        for f in todo:
            f()
        return 0

    if SCOPES:
        def phase_s(j, c):
            with jax.named_scope("ph"):
                return phase(j, c)
        jax.lax.fori_loop(0, _HQ, phase_s, 0)
    else:
        jax.lax.fori_loop(0, _HQ, phase, 0)

    n_lo = len(ffn_lo)
    done = [0]

    def ticks_to(n):
        for i in range(done[0], n + 1):
            if SCOPES:
                with jax.named_scope(f"w{i}"):
                    ffn_lo_copy(i).wait()
            else:
                ffn_lo_copy(i).wait()
            if i < len(ffn_hi):
                ffn_hi_copy(i).start(priority=_HI)
            if i + n_half < n_lo:
                ffn_lo_copy(i + n_half).start(priority=_LO)
        done[0] = max(done[0], n + 1)

    last = (_HQ - 1) & 1
    carry = pv_init()
    for i in range(PV_SL):
        ticks_to(i * 12 // PV_SL)
        carry = pv_slice(last, i, carry)
    ticks_to(12)
    hres = attn_v[...] + out_proj(last, pv_finish(*carry))
    ticks_to(13)
    hn = _layernorm(hres).astype(bf16)

    n_w1 = (d_model - w1_hi) // 32
    n_w3 = w3_lo // 32
    ticks_to(n_w1 - 1)
    wait_all(w1_v.at[pl.ds(0, w1_hi), :], sem_f0.at[0])
    gates = []
    for s in range(4):
        gates.append(jnp.dot(hn, w1_v[:, s * _PAIR:(s + 1) * _PAIR],
                             preferred_element_type=f32))
        ticks_to(n_w1 + s + (s + 1) // 2)
    gate = jnp.concatenate(gates, axis=-1)
    gate = gate * jax.nn.sigmoid(gate)

    def up_chunk(c):
        return jnp.dot(hn[:, c * 128:(c + 1) * 128], w3_v[c * 128:(c + 1) * 128, :],
                       preferred_element_type=f32)

    up = up_chunk(0)
    ticks_to(n_w1 + 7)
    up = up + up_chunk(1)
    ticks_to(n_w1 + 11)
    up = up + up_chunk(2)
    ticks_to(n_w1 + 12)
    wait_all(w3_v.at[pl.ds(w3_lo, d_model - w3_lo), :], sem_f0.at[1])
    up = up + up_chunk(4)
    ticks_to(n_w1 + n_w3 - 1)
    up = up + up_chunk(3)
    act = (gate * up).astype(bf16)

    def down(r0, n):
        return jnp.dot(act[:, r0:r0 + n], w2_v[r0:r0 + n, :], preferred_element_type=f32)

    out = hres
    first_w2 = n_w1 + n_w3
    for k in range(1, n_lo - first_w2, 2):
        ticks_to(first_w2 + k)
        out = out + down(_W2_HI + (k - 1) * 64, 128)
        if first_w2 + k == n_lo - 5:
            wait_all(w2_v.at[pl.ds(0, _W2_HI), :], sem_f0.at[2])
            out = out + down(0, _W2_HI)
    assert done[0] == n_lo
    o_ref[...] = out[0:1, :].astype(o_ref.dtype)


@jax.jit
def pallas_sequential_preLN__sliding_block_cached__glu_gated_swiglu__decode_kernel(
    A_x: jax.Array,
    A_k_cache: jax.Array,
    A_v_cache: jax.Array,
    A_wq: jax.Array,
    A_wo: jax.Array,
    B_x: jax.Array,
    B_w1: jax.Array,
    B_w3: jax.Array,
    B_w2: jax.Array,
):
    del B_x
    b, sq, d_model = A_x.shape
    hkv, sk = A_k_cache.shape[1], A_k_cache.shape[2]
    d_ff = B_w1.shape[1]
    assert b == 1 and sq == 1 and hkv == _HQ and A_k_cache.shape[3] == _DH
    win = min(4096, max(256, sk // 4))
    bf16, f32 = jnp.bfloat16, jnp.float32

    k_t = jnp.swapaxes(A_k_cache, 2, 3)
    v_t = jnp.swapaxes(A_v_cache, 2, 3)
    x2 = A_x.reshape(1, d_model)
    wo3 = A_wo.reshape(_HQ, _DH, d_model)

    any_spec = pl.BlockSpec(memory_space=pl.ANY)
    dma = pltpu.SemaphoreType.DMA
    out = pl.pallas_call(
        functools.partial(_kernel, win_start=sk - win, win=win),
        out_shape=jax.ShapeDtypeStruct((1, d_model), A_x.dtype),
        in_specs=[any_spec] * 8,
        out_specs=pl.BlockSpec(memory_space=pltpu.VMEM),
        scratch_shapes=[
            pltpu.VMEM((1, d_model), bf16),
            pltpu.VMEM((_ROWS, d_model), bf16),
            pltpu.VMEM((2, d_model, _PAIR), bf16),
            pltpu.VMEM((2, _DH, d_model), bf16),
            pltpu.VMEM((d_model, d_ff), bf16),
            pltpu.VMEM((d_model, d_ff), bf16),
            pltpu.VMEM((d_ff, d_model), bf16),
            pltpu.VMEM((2, _DH, win), bf16),
            pltpu.VMEM((2, _DH, win), bf16),
            pltpu.VMEM((2, _ROWS, _DH), bf16),
            pltpu.VMEM((_ROWS, win), f32),
            pltpu.VMEM((_ROWS, 128), f32),
            pltpu.VMEM((_ROWS, _DH), bf16),
            pltpu.VMEM((_ROWS, d_model), f32),
            dma((1,)), dma((2,)), dma((2,)), dma((2,)), dma((2,)),
            dma((50,)), dma((3,)),
        ],
        compiler_params=pltpu.CompilerParams(
            vmem_limit_bytes=48 * 1024 * 1024, disable_semaphore_checks=True,
            disable_bounds_checks=not BOUNDS),
    )(x2, k_t, v_t, A_wq, wo3, B_w1, B_w3, B_w2)
    return out.reshape(b, sq, d_model)
```

```python
import functools

import jax
import jax.numpy as jnp
import jax.experimental.pallas as pl
import jax.experimental.pallas.tpu as pltpu

_HQ = 32
_DH = 192
_EPS = 1e-5
_ROWS = 8
_PAIR = 2 * _DH
_HI, _LO = 0, 1
_GRP = 4

KV_W = (640, 640, 640, 640, 640, 896)
KV_R = 32
RBQ = 8
RBO = 8
LOOK = 20
PV_SL = 8
QK_SL = 8
W2_HI = 256
LAST = 128
LAND = 15
W2_G = 256
BOUNDS = False
SCOPES = False


def _layernorm(x):
    m = jnp.mean(x, axis=-1, keepdims=True)
    c = x - m
    v = jnp.mean(c * c, axis=-1, keepdims=True)
    return c / jnp.sqrt(v + _EPS)


def _kernel(x_hbm, k_hbm, v_hbm, wq_hbm, wo_hbm, w1_hbm, w3_hbm, w2_hbm, o_ref,
            x_v, xn_v, wq_v, wo_v, w1_v, w3_v, w2_v, kbuf, vbuf, q_v, s_v, m_v, av_v, attn_v,
            sem_x, sem_wq, sem_k, sem_v, sem_wo, sem_f1, sem_f0,
            *, win_start, win):
    f32, bf16 = jnp.float32, jnp.bfloat16
    d_model = x_v.shape[-1]
    d_ff = w1_v.shape[-1]
    n_rb = _DH // KV_R
    assert sum(KV_W) == win
    n = n_rb * len(KV_W)
    n_wq = d_model // RBQ // _GRP
    n_wo = 2 * (_DH // RBO)
    wo_cols = ((0, 256), (256, d_model - 256))
    assert n_wq + n_wo <= 2 * n and LOOK <= n and n_wq % 2 == 0
    assert d_ff == 4 * _PAIR and d_model % 128 == 0
    scale = _DH ** -0.5

    def ds(start, size, align):
        if isinstance(start, int):
            return pl.ds(start, size)
        return pl.ds(pl.multiple_of(start, align), size)

    def kv_copy(hbm, buf, sem, h, slot, t):
        rows = pl.ds((t % n_rb) * KV_R, KV_R)
        c, w = sum(KV_W[:t // n_rb]), KV_W[t // n_rb]
        return pltpu.make_async_copy(
            hbm.at[0, h, rows, pl.ds(win_start + c, w)],
            buf.at[slot, rows, pl.ds(c, w)], sem.at[slot])

    k_copy = functools.partial(kv_copy, k_hbm, kbuf, sem_k)
    v_copy = functools.partial(kv_copy, v_hbm, vbuf, sem_v)

    def wq_copy(grp, slot, r0, nrows):
        rows = ds(r0, nrows, 8)
        return pltpu.make_async_copy(
            wq_hbm.at[rows, ds(grp * (_GRP * _DH), _GRP * _DH, 128)],
            wq_v.at[slot, rows, :], sem_wq.at[slot])

    def wo_copy(h, slot, b):
        rows, cols = pl.ds((b // 2) * RBO, RBO), pl.ds(*wo_cols[b % 2])
        return pltpu.make_async_copy(wo_hbm.at[h, rows, cols], wo_v.at[slot, rows, cols],
                                     sem_wo.at[slot])

    def block_copy(hbm, buf, r0, nrows, c0, ncols, sem):
        rows, cols = ds(r0, nrows, 8), pl.ds(c0, ncols)
        return pltpu.make_async_copy(hbm.at[rows, cols], buf.at[rows, cols], sem)

    def wait_all(ref, sem):
        pltpu.make_async_copy(ref, ref, sem).wait()

    w1_hi = d_model // 2
    w3_lo = d_model - d_model // 4
    w2_groups = []
    r = W2_HI
    while r < d_ff:
        left = d_ff - r
        nr = W2_G if left >= W2_G + 2 * 128 else min(128, left)
        if r + nr == d_ff and nr > LAST:
            nr -= LAST
        w2_groups.append((r, nr))
        r += nr
    ffn_lo = ([(w1_hbm, w1_v, r, 16, 0, d_ff, 0) for r in range(w1_hi, d_model, 16)]
              + [(w3_hbm, w3_v, r, 16, 0, d_ff, 1 + r // 128) for r in range(0, w3_lo, 16)]
              + [(w2_hbm, w2_v, r, 32, 0, d_model, 5 + gi)
                 for gi, (r0, nr) in enumerate(w2_groups) for r in range(r0, r0 + nr, 32)])
    ffn_hi = ([(w3_hbm, w3_v, r, 8, c, d_ff // 2, 1)
               for r in range(w3_lo, d_model, 8) for c in (0, d_ff // 2)]
              + [(w2_hbm, w2_v, r, 8, 0, d_model, 2 + r // 128) for r in range(0, W2_HI, 8)])

    def ffn_lo_copy(i):
        return block_copy(*ffn_lo[i][:6], sem_f1.at[ffn_lo[i][6]])

    def ffn_hi_copy(i):
        return block_copy(*ffn_hi[i][:6], sem_f0.at[ffn_hi[i][6]])

    def qk_slice(slot, i, mx):
        w = win // QK_SL
        cols = pl.ds(i * w, w)
        s = jnp.dot(q_v[slot], kbuf[slot, :, cols], preferred_element_type=f32) * scale
        s_v[:, cols] = s
        for c in range(w // 128):
            mx = jnp.maximum(mx, s[:, c * 128:(c + 1) * 128])
        return mx

    def pv_slice(slot, i, carry):
        w = win // PV_SL
        acc, den = carry
        cols = pl.ds(i * w, w)
        p = jnp.exp(s_v[:, cols] - jnp.concatenate([m_v[...]] * (w // 128), axis=-1))
        for c in range(w // 128):
            den = den + p[:, c * 128:(c + 1) * 128]
        acc = acc + jax.lax.dot_general(
            p.astype(bf16), vbuf[slot, :, cols], (((1,), (1,)), ((), ())),
            preferred_element_type=f32)
        return acc, den

    def pv_init():
        return jnp.zeros((_ROWS, _DH), f32), jnp.zeros((_ROWS, 128), f32)

    def pv_finish(acc, den):
        return (acc / jnp.sum(den, axis=-1, keepdims=True)).astype(bf16)

    def out_proj(slot, o):
        wait_all(wo_v.at[slot], sem_wo.at[slot])
        return jnp.dot(o, wo_v[slot], preferred_element_type=f32)

    def q_proj(slot, half):
        w = wq_v[slot, :, pl.ds(pl.multiple_of(half * _PAIR, 128), _PAIR)]
        q = jnp.dot(xn_v[...], w, preferred_element_type=f32).astype(bf16)
        q_v[0] = q[:, :_DH]
        q_v[1] = q[:, _DH:]

    x_copy = pltpu.make_async_copy(x_hbm, x_v, sem_x.at[0])
    x_copy.start(priority=_HI)
    for r in range(0, d_model, 128):
        wq_copy(0, 0, r, 128).start(priority=_LO)
    for t in range(LOOK):
        k_copy(0, 0, t).start(priority=_LO)
    x_copy.wait()
    x = jnp.broadcast_to(x_v[...].astype(f32), (_ROWS, d_model))
    xn_v[...] = _layernorm(x).astype(bf16)
    attn_v[...] = x

    pieces = sorted([((i + 0.5) / n_wq, "q", i) for i in range(n_wq)]
                    + [((i + 0.5) / n_wo, "o", i) for i in range(n_wo)])
    piece_at = {(i * 2 * n) // len(pieces): p[1:] for i, p in enumerate(pieces)}

    def phase(j, _):
        slot = j & 1
        prev = 1 - slot
        grp = (j >> 2) + 1
        gslot = grp & 1
        quarter = j & (_GRP - 1)

        def start_piece(t):
            if t not in piece_at:
                return
            kind, b = piece_at[t]
            if kind == "o":
                wo_copy(j, slot, b).start(priority=_HI)
                return

            @pl.when(j < _HQ - _GRP)
            def _():
                wq_copy(grp, gslot, (quarter * n_wq + b) * RBQ, RBQ).start(priority=_HI)

            @pl.when(j >= _HQ - _GRP)
            def _():
                block_copy(w1_hbm, w1_v, (quarter * (n_wq // 2) + b // 2) * RBQ, RBQ,
                           (b % 2) * (d_ff // 2), d_ff // 2,
                           sem_f0.at[0]).start(priority=_HI)

        def tick(t):
            if t < n:
                k_copy(j, slot, t).wait()
            else:
                v_copy(j, slot, t - n).wait()
            start_piece(t)
            u = t + LOOK
            if u < n:
                k_copy(j, slot, u).start(priority=_LO)
            elif u < 2 * n:
                v_copy(j, slot, u - n).start(priority=_LO)
            else:
                @pl.when(j + 1 < _HQ)
                def _():
                    k_copy(j + 1, prev, u - 2 * n).start(priority=_LO)

                @pl.when(j + 1 == _HQ)
                def _():
                    ffn_lo_copy(u - 2 * n).start(priority=_LO)

        g = n // PV_SL
        t_q = min(g * PV_SL, n - 1)

        def maybe_q(t):
            if t == t_q:
                @pl.when(quarter == 0)
                def _():
                    wait_all(wq_v.at[1 - gslot], sem_wq.at[1 - gslot])

                @pl.when(slot == 0)
                def _():
                    q_proj(1 - gslot, quarter >> 1)

        @pl.when(j > 0)
        def _():
            carry = pv_init()
            for t in range(n):
                tick(t)
                if t % g == 0 and t // g < PV_SL:
                    carry = pv_slice(prev, t // g, carry)
                maybe_q(t)
            av_v[...] = pv_finish(*carry)

        @pl.when(j == 0)
        def _():
            for t in range(n):
                tick(t)
                maybe_q(t)

        gq = (n - 1) // QK_SL
        mx = jnp.full((_ROWS, 128), -jnp.inf, f32)
        for t in range(n):
            tick(n + t)
            if t % gq == 0 and t // gq < QK_SL:
                mx = qk_slice(slot, t // gq, mx)
            if t == gq * QK_SL:
                m_v[...] = jnp.broadcast_to(jnp.max(mx, axis=-1, keepdims=True), (_ROWS, 128))

                @pl.when(j > 0)
                def _():
                    attn_v[...] += out_proj(prev, av_v[...])
        return 0

    if SCOPES:
        def phase_s(j, c):
            with jax.named_scope("ph"):
                return phase(j, c)
        jax.lax.fori_loop(0, _HQ, phase_s, 0)
    else:
        jax.lax.fori_loop(0, _HQ, phase, 0)

    n_lo = len(ffn_lo)
    done = [0]

    def ticks_to(m):
        for i in range(done[0], m + 1):
            if SCOPES:
                with jax.named_scope(f"w{i}"):
                    ffn_lo_copy(i).wait()
            else:
                ffn_lo_copy(i).wait()
            if i < len(ffn_hi):
                ffn_hi_copy(i).start(priority=_HI)
            if i + LOOK < n_lo:
                ffn_lo_copy(i + LOOK).start(priority=_LO)
        done[0] = max(done[0], m + 1)

    def lo_done(group):
        return max(i for i, e in enumerate(ffn_lo) if e[6] == group)

    def hi_done(group):
        return max(i for i, e in enumerate(ffn_hi) if e[6] == group) + LAND

    last = (_HQ - 1) & 1
    carry = pv_init()
    for i in range(PV_SL):
        ticks_to(i * 18 // PV_SL)
        carry = pv_slice(last, i, carry)
    ticks_to(18)
    hres = attn_v[...] + out_proj(last, pv_finish(*carry))
    ticks_to(21)
    hn = _layernorm(hres).astype(bf16)

    t0 = max(lo_done(0), 23)
    ticks_to(t0)
    wait_all(w1_v.at[pl.ds(0, w1_hi), :], sem_f0.at[0])
    gates = []
    for s in range(4):
        gates.append(jnp.dot(hn, w1_v[:, s * _PAIR:(s + 1) * _PAIR],
                             preferred_element_type=f32))
        ticks_to(t0 + (5 * (s + 1)) // 2)
    gate = jnp.concatenate(gates, axis=-1)
    gate = gate * jax.nn.sigmoid(gate)

    def up_chunk(c):
        return jnp.dot(hn[:, c * 128:(c + 1) * 128], w3_v[c * 128:(c + 1) * 128, :],
                       preferred_element_type=f32)

    ticks_to(lo_done(1))
    up = up_chunk(0)
    ticks_to(lo_done(2))
    up = up + up_chunk(1)
    ticks_to(lo_done(3))
    up = up + up_chunk(2)
    ticks_to(hi_done(1) + 1)
    wait_all(w3_v.at[pl.ds(w3_lo, d_model - w3_lo), :], sem_f0.at[1])
    up = up + up_chunk(4)
    ticks_to(lo_done(4))
    up = up + up_chunk(3)
    act = (gate * up).astype(bf16)

    hi_groups = [(c * 128, min(128, W2_HI - c * 128)) for c in range(-(-W2_HI // 128))]
    lhs = {g: act[:, g[0]:g[0] + g[1]] for g in w2_groups + hi_groups}

    def down(g):
        return jnp.dot(lhs[g], w2_v[g[0]:g[0] + g[1], :], preferred_element_type=f32)

    out = hres
    pending = list(enumerate(hi_groups))
    for gi, g in enumerate(w2_groups):
        ticks_to(lo_done(5 + gi))
        part = down(g)
        if pending and hi_done(2 + pending[0][0]) <= lo_done(5 + gi):
            c, hg = pending.pop(0)
            wait_all(w2_v.at[pl.ds(hg[0], hg[1]), :], sem_f0.at[2 + c])
            part = part + down(hg)
        out = out + part
    assert done[0] == n_lo and not pending
    o_ref[...] = out[0:1, :].astype(o_ref.dtype)


@jax.jit
def pallas_sequential_preLN__sliding_block_cached__glu_gated_swiglu__decode_kernel(
    A_x: jax.Array,
    A_k_cache: jax.Array,
    A_v_cache: jax.Array,
    A_wq: jax.Array,
    A_wo: jax.Array,
    B_x: jax.Array,
    B_w1: jax.Array,
    B_w3: jax.Array,
    B_w2: jax.Array,
):
    del B_x
    b, sq, d_model = A_x.shape
    hkv, sk = A_k_cache.shape[1], A_k_cache.shape[2]
    d_ff = B_w1.shape[1]
    assert b == 1 and sq == 1 and hkv == _HQ and A_k_cache.shape[3] == _DH
    win = min(4096, max(256, sk // 4))
    bf16, f32 = jnp.bfloat16, jnp.float32

    k_t = jnp.swapaxes(A_k_cache, 2, 3)
    v_t = jnp.swapaxes(A_v_cache, 2, 3)
    x2 = A_x.reshape(1, d_model)
    wo3 = A_wo.reshape(_HQ, _DH, d_model)

    any_spec = pl.BlockSpec(memory_space=pl.ANY)
    dma = pltpu.SemaphoreType.DMA
    out = pl.pallas_call(
        functools.partial(_kernel, win_start=sk - win, win=win),
        out_shape=jax.ShapeDtypeStruct((1, d_model), A_x.dtype),
        in_specs=[any_spec] * 8,
        out_specs=pl.BlockSpec(memory_space=pltpu.VMEM),
        scratch_shapes=[
            pltpu.VMEM((1, d_model), bf16),
            pltpu.VMEM((_ROWS, d_model), bf16),
            pltpu.VMEM((2, d_model, _GRP * _DH), bf16),
            pltpu.VMEM((2, _DH, d_model), bf16),
            pltpu.VMEM((d_model, d_ff), bf16),
            pltpu.VMEM((d_model, d_ff), bf16),
            pltpu.VMEM((d_ff, d_model), bf16),
            pltpu.VMEM((2, _DH, win), bf16),
            pltpu.VMEM((2, _DH, win), bf16),
            pltpu.VMEM((2, _ROWS, _DH), bf16),
            pltpu.VMEM((_ROWS, win), f32),
            pltpu.VMEM((_ROWS, 128), f32),
            pltpu.VMEM((_ROWS, _DH), bf16),
            pltpu.VMEM((_ROWS, d_model), f32),
            dma((1,)), dma((2,)), dma((2,)), dma((2,)), dma((2,)),
            dma((18,)), dma((6,)),
        ],
        compiler_params=pltpu.CompilerParams(
            vmem_limit_bytes=48 * 1024 * 1024, disable_semaphore_checks=True,
            disable_bounds_checks=not BOUNDS),
    )(x2, k_t, v_t, A_wq, wo3, B_w1, B_w3, B_w2)
    return out.reshape(b, sq, d_model)
```

```python
import functools

import jax
import jax.numpy as jnp
import jax.experimental.pallas as pl
import jax.experimental.pallas.tpu as pltpu

_HQ = 32
_DH = 192
_EPS = 1e-5
_ROWS = 8
_PAIR = 2 * _DH
_HI, _LO = 0, 1
_GRP = 4

KV_W = (640,640,640,640,768,768)
KV_R = 32
RBQ = 8
RBO = 8
LOOK = 24
PV_SL = 8
QK_SL = 8
W2_HI = 256
LAST = 128
LAND = 15
W2_G = 256
PRE = 2
WQ0_R = 32
T_LN = 2
BOUNDS = True
SCOPES = False
VPU_R = 256
VPU_D = 32


def _layernorm(x):
    m = jnp.mean(x, axis=-1, keepdims=True)
    c = x - m
    v = jnp.mean(c * c, axis=-1, keepdims=True)
    return c / jnp.sqrt(v + _EPS)


def _kernel(x_hbm, k_hbm, v_hbm, wq_hbm, wo_hbm, w1_hbm, w3_hbm, w2_hbm, o_ref,
            x_v, xn_v, wq_v, wo_v, w1_v, w3_v, w2_v, kbuf, vbuf, q_v, s_v, m_v, av_v, attn_v,
            sem_x, sem_wq, sem_k, sem_v, sem_wo, sem_f1, sem_f0,
            *, win_start, win):
    f32, bf16 = jnp.float32, jnp.bfloat16
    d_model = x_v.shape[-1]
    d_ff = w1_v.shape[-1]
    n_rb = _DH // KV_R
    assert sum(KV_W) == win
    n = n_rb * len(KV_W)
    n_wq = d_model // RBQ // _GRP
    n_wo = 2 * (_DH // RBO)
    wo_cols = ((0, 256), (256, d_model - 256))
    assert n_wq + n_wo <= 2 * n and LOOK <= n and n_wq % 2 == 0
    assert d_ff == 4 * _PAIR and d_model % 128 == 0
    scale = _DH ** -0.5

    def ds(start, size, align):
        if isinstance(start, int):
            return pl.ds(start, size)
        return pl.ds(pl.multiple_of(start, align), size)

    def kv_copy(hbm, buf, sem, h, slot, t):
        rows = pl.ds((t % n_rb) * KV_R, KV_R)
        c, w = sum(KV_W[:t // n_rb]), KV_W[t // n_rb]
        return pltpu.make_async_copy(
            hbm.at[0, h, rows, pl.ds(win_start + c, w)],
            buf.at[slot, rows, pl.ds(c, w)], sem.at[slot])

    k_copy = functools.partial(kv_copy, k_hbm, kbuf, sem_k)
    v_copy = functools.partial(kv_copy, v_hbm, vbuf, sem_v)

    def wq_copy(grp, slot, r0, nrows):
        rows = ds(r0, nrows, 8)
        return pltpu.make_async_copy(
            wq_hbm.at[rows, ds(grp * (_GRP * _DH), _GRP * _DH, 128)],
            wq_v.at[slot, rows, :], sem_wq.at[slot])

    def wo_copy(h, slot, b):
        rows, cols = pl.ds((b // 2) * RBO, RBO), pl.ds(*wo_cols[b % 2])
        return pltpu.make_async_copy(wo_hbm.at[h, rows, cols], wo_v.at[slot, rows, cols],
                                     sem_wo.at[slot])

    def block_copy(hbm, buf, r0, nrows, c0, ncols, sem):
        rows, cols = ds(r0, nrows, 8), pl.ds(c0, ncols)
        return pltpu.make_async_copy(hbm.at[rows, cols], buf.at[rows, cols], sem)

    def wait_all(ref, sem):
        pltpu.make_async_copy(ref, ref, sem).wait()

    w1_hi = d_model // 2
    w3_lo = d_model - d_model // 4
    w2_groups = []
    r = W2_HI
    mxu_end = d_ff - VPU_R
    while r < mxu_end:
        left = mxu_end - r
        nr = W2_G if left >= W2_G + 2 * 128 else min(128, left)
        w2_groups.append((r, nr))
        r += nr
    ffn_lo = ([(w1_hbm, w1_v, r, 16, 0, d_ff, 0) for r in range(w1_hi, d_model, 16)]
              + [(w3_hbm, w3_v, r, 16, 0, d_ff, 1 + r // 128) for r in range(0, w3_lo, 16)]
              + [(w2_hbm, w2_v, r, 32, 0, d_model, 5 + gi)
                 for gi, (r0, nr) in enumerate(w2_groups) for r in range(r0, r0 + nr, 32)]
              + [(w2_hbm, w2_v, r, VPU_D, 0, d_model, 5 + len(w2_groups) + i)
                 for i, r in enumerate(range(mxu_end, d_ff, VPU_D))])
    ffn_hi = ([(w3_hbm, w3_v, r, 8, c, d_ff // 2, 1)
               for r in range(w3_lo, d_model, 8) for c in (0, d_ff // 2)]
              + [(w2_hbm, w2_v, r, 8, 0, d_model, 2 + r // 128) for r in range(0, W2_HI, 8)])

    def ffn_lo_copy(i):
        return block_copy(*ffn_lo[i][:6], sem_f1.at[ffn_lo[i][6]])

    def ffn_hi_copy(i):
        return block_copy(*ffn_hi[i][:6], sem_f0.at[ffn_hi[i][6]])

    def qk_slice(slot, i, mx):
        w = win // QK_SL
        cols = pl.ds(i * w, w)
        s = jnp.dot(q_v[slot], kbuf[slot, :, cols], preferred_element_type=f32) * scale
        s_v[:, cols] = s
        for c in range(w // 128):
            mx = jnp.maximum(mx, s[:, c * 128:(c + 1) * 128])
        return mx

    def pv_slice(slot, i, carry):
        w = win // PV_SL
        acc, den = carry
        cols = pl.ds(i * w, w)
        p = jnp.exp(s_v[:, cols] - jnp.concatenate([m_v[...]] * (w // 128), axis=-1))
        for c in range(w // 128):
            den = den + p[:, c * 128:(c + 1) * 128]
        acc = acc + jax.lax.dot_general(
            p.astype(bf16), vbuf[slot, :, cols], (((1,), (1,)), ((), ())),
            preferred_element_type=f32)
        return acc, den

    def pv_init():
        return jnp.zeros((_ROWS, _DH), f32), jnp.zeros((_ROWS, 128), f32)

    def pv_finish(acc, den):
        return (acc / jnp.sum(den, axis=-1, keepdims=True)).astype(bf16)

    def out_proj(slot, o):
        wait_all(wo_v.at[slot], sem_wo.at[slot])
        return jnp.dot(o, wo_v[slot], preferred_element_type=f32)

    def q_proj(slot, half):
        w = wq_v[slot, :, ds(half * _PAIR, _PAIR, 128)]
        q = jnp.dot(xn_v[...], w, preferred_element_type=f32).astype(bf16)
        q_v[0] = q[:, :_DH]
        q_v[1] = q[:, _DH:]

    pieces = sorted([((i + 0.5) / n_wq, "q", i) for i in range(n_wq)]
                    + [((i + 0.5) / n_wo, "o", i) for i in range(n_wo)])
    piece_at = {(i * 2 * n) // len(pieces): p[1:] for i, p in enumerate(pieces)}

    n_a = sum(1 for t in piece_at if t < n)

    def start_hi(j, kind, b):
        slot, quarter = j & 1, j & (_GRP - 1)
        grp = (j >> 2) + 1
        if kind == "o":
            wo_copy(j, slot, b).start(priority=_HI)
        elif isinstance(j, int):
            wq_copy(grp, grp & 1, (quarter * n_wq + b) * RBQ, RBQ).start(priority=_HI)
        else:
            @pl.when(j < _HQ - _GRP)
            def _():
                wq_copy(grp, grp & 1, (quarter * n_wq + b) * RBQ, RBQ).start(priority=_HI)

            @pl.when(j >= _HQ - _GRP)
            def _():
                block_copy(w1_hbm, w1_v, (quarter * (n_wq // 2) + b // 2) * RBQ, RBQ,
                           (b % 2) * (d_ff // 2), d_ff // 2,
                           sem_f0.at[0]).start(priority=_HI)

    x_copy = pltpu.make_async_copy(x_hbm, x_v, sem_x.at[0])
    seq0 = ([k_copy(0, 0, t) for t in range(n)]
            + [wq_copy(0, 0, r, WQ0_R) for r in range(0, d_model, WQ0_R)])
    n0 = len(seq0)
    seq0 += [v_copy(0, 0, t) for t in range(LOOK)]
    hi0 = [p[1:] for p in pieces[:n_a]]
    hi0_at = {(i * n0) // (n_a - PRE): p for i, p in enumerate(hi0[PRE:])}
    x_copy.start(priority=_HI)
    for c in seq0[:LOOK]:
        c.start(priority=_LO)
    for p in hi0[:PRE]:
        start_hi(0, *p)
    for t in range(n0):
        seq0[t].wait()
        if t in hi0_at:
            start_hi(0, *hi0_at[t])
        seq0[t + LOOK].start(priority=_LO)
        if t == T_LN:
            x_copy.wait()
            x = jnp.broadcast_to(x_v[...].astype(f32), (_ROWS, d_model))
            xn_v[...] = _layernorm(x).astype(bf16)
            attn_v[...] = x
    q_proj(0, 0)

    def phase(j, _):
        slot = j & 1
        prev = 1 - slot
        gslot = (j >> 2) & 1
        quarter = j & (_GRP - 1)

        def tick(t):
            if t < n:
                k_copy(j, slot, t).wait()
            else:
                v_copy(j, slot, t - n).wait()
            if t in piece_at:
                start_hi(j, *piece_at[t])
            u = t + LOOK
            if u < n:
                k_copy(j, slot, u).start(priority=_LO)
            elif u < 2 * n:
                v_copy(j, slot, u - n).start(priority=_LO)
            else:
                @pl.when(j + 1 < _HQ)
                def _():
                    k_copy(j + 1, prev, u - 2 * n).start(priority=_LO)

                @pl.when(j + 1 == _HQ)
                def _():
                    ffn_lo_copy(u - 2 * n).start(priority=_LO)

        g = n // PV_SL
        t_q = min(g * PV_SL, n - 1)

        def maybe_q(t):
            if t == t_q:
                @pl.when(quarter == 0)
                def _():
                    wait_all(wq_v.at[gslot], sem_wq.at[gslot])

                @pl.when(slot == 0)
                def _():
                    q_proj(gslot, quarter >> 1)

        @pl.when(j > 0)
        def _():
            carry = pv_init()
            for t in range(n):
                tick(t)
                if t % g == 0 and t // g < PV_SL:
                    carry = pv_slice(prev, t // g, carry)
                maybe_q(t)
            av_v[...] = pv_finish(*carry)

        gq = (n - 1) // QK_SL
        mx = jnp.full((_ROWS, 128), -jnp.inf, f32)
        for t in range(n):
            tick(n + t)
            if t % gq == 0 and t // gq < QK_SL:
                mx = qk_slice(slot, t // gq, mx)
            if t == gq * QK_SL:
                m_v[...] = jnp.broadcast_to(jnp.max(mx, axis=-1, keepdims=True), (_ROWS, 128))

                @pl.when(j > 0)
                def _():
                    attn_v[...] += out_proj(prev, av_v[...])
        return 0

    if SCOPES:
        def phase_s(j, c):
            with jax.named_scope("ph"):
                return phase(j, c)
        jax.lax.fori_loop(0, _HQ, phase_s, 0)
    else:
        jax.lax.fori_loop(0, _HQ, phase, 0)

    n_lo = len(ffn_lo)
    done = [0]

    def ticks_to(m):
        for i in range(done[0], m + 1):
            if SCOPES:
                with jax.named_scope(f"w{i}"):
                    ffn_lo_copy(i).wait()
            else:
                ffn_lo_copy(i).wait()
            if i < len(ffn_hi):
                ffn_hi_copy(i).start(priority=_HI)
            if i + LOOK < n_lo:
                ffn_lo_copy(i + LOOK).start(priority=_LO)
        done[0] = max(done[0], m + 1)

    def lo_done(group):
        return max(i for i, e in enumerate(ffn_lo) if e[6] == group)

    def hi_done(group):
        return max(i for i, e in enumerate(ffn_hi) if e[6] == group) + LAND

    last = (_HQ - 1) & 1
    carry = pv_init()
    for i in range(PV_SL):
        ticks_to(i * 18 // PV_SL)
        carry = pv_slice(last, i, carry)
    ticks_to(18)
    hres = attn_v[...] + out_proj(last, pv_finish(*carry))
    ticks_to(21)
    hn = _layernorm(hres).astype(bf16)

    t0 = max(lo_done(0), 23)
    ticks_to(t0)
    wait_all(w1_v.at[pl.ds(0, w1_hi), :], sem_f0.at[0])
    gates = []
    for s in range(4):
        gates.append(jnp.dot(hn, w1_v[:, s * _PAIR:(s + 1) * _PAIR],
                             preferred_element_type=f32))
        ticks_to(t0 + (5 * (s + 1)) // 2)
    gate = jnp.concatenate(gates, axis=-1)
    gate = gate * jax.nn.sigmoid(gate)

    def up_chunk(c):
        return jnp.dot(hn[:, c * 128:(c + 1) * 128], w3_v[c * 128:(c + 1) * 128, :],
                       preferred_element_type=f32)

    ticks_to(lo_done(1))
    up = up_chunk(0)
    ticks_to(lo_done(2))
    up = up + up_chunk(1)
    ticks_to(lo_done(3))
    up = up + up_chunk(2)
    ticks_to(hi_done(1) + 1)
    wait_all(w3_v.at[pl.ds(w3_lo, d_model - w3_lo), :], sem_f0.at[1])
    up = up + up_chunk(4)
    ticks_to(lo_done(4))
    up = up + up_chunk(3)
    act = (gate * up).astype(bf16)

    hi_groups = [(c * 128, min(128, W2_HI - c * 128)) for c in range(-(-W2_HI // 128))]
    lhs = {g: act[:, g[0]:g[0] + g[1]] for g in w2_groups + hi_groups}

    def down(g):
        return jnp.dot(lhs[g], w2_v[g[0]:g[0] + g[1], :], preferred_element_type=f32)

    if VPU_R:
        col0 = (mxu_end // 128) * 128
        act_col = jnp.concatenate(
            [jnp.broadcast_to(act[0:1, c:c + 128].astype(f32), (128, 128)).T
             for c in range(col0, d_ff, 128)], axis=0)
    out = hres
    pending = list(enumerate(hi_groups))
    for gi, g in enumerate(w2_groups):
        ticks_to(lo_done(5 + gi))
        part = down(g)
        while pending and (hi_done(2 + pending[0][0]) <= lo_done(5 + gi)
                           or gi == len(w2_groups) - 1):
            c, hg = pending.pop(0)
            wait_all(w2_v.at[pl.ds(hg[0], hg[1]), :], sem_f0.at[2 + c])
            part = part + down(hg)
        out = out + part
    assert not pending
    res = out[0:1, :]
    if VPU_R:
        tail = jnp.zeros((8, d_model), f32)
        for i, r in enumerate(range(mxu_end, d_ff, VPU_D)):
            ticks_to(lo_done(5 + len(w2_groups) + i))
            a = act_col[r - col0:r - col0 + VPU_D, :]
            prod = w2_v[r:r + VPU_D, :].astype(f32) * jnp.concatenate(
                [a] * (d_model // 128), axis=-1)
            for k in range(VPU_D // 8):
                tail = tail + prod[k * 8:(k + 1) * 8, :]
        res = res + jnp.sum(tail, axis=0, keepdims=True)
    assert done[0] == n_lo
    o_ref[...] = res.astype(o_ref.dtype)


@jax.jit
def pallas_sequential_preLN__sliding_block_cached__glu_gated_swiglu__decode_kernel(
    A_x: jax.Array,
    A_k_cache: jax.Array,
    A_v_cache: jax.Array,
    A_wq: jax.Array,
    A_wo: jax.Array,
    B_x: jax.Array,
    B_w1: jax.Array,
    B_w3: jax.Array,
    B_w2: jax.Array,
):
    del B_x
    b, sq, d_model = A_x.shape
    hkv, sk = A_k_cache.shape[1], A_k_cache.shape[2]
    d_ff = B_w1.shape[1]
    assert b == 1 and sq == 1 and hkv == _HQ and A_k_cache.shape[3] == _DH
    win = min(4096, max(256, sk // 4))
    bf16, f32 = jnp.bfloat16, jnp.float32

    k_t = jnp.swapaxes(A_k_cache, 2, 3)
    v_t = jnp.swapaxes(A_v_cache, 2, 3)
    x2 = A_x.reshape(1, d_model)
    wo3 = A_wo.reshape(_HQ, _DH, d_model)

    any_spec = pl.BlockSpec(memory_space=pl.ANY)
    dma = pltpu.SemaphoreType.DMA
    out = pl.pallas_call(
        functools.partial(_kernel, win_start=sk - win, win=win),
        out_shape=jax.ShapeDtypeStruct((1, d_model), A_x.dtype),
        in_specs=[any_spec] * 8,
        out_specs=pl.BlockSpec(memory_space=pltpu.VMEM),
        scratch_shapes=[
            pltpu.VMEM((1, d_model), bf16),
            pltpu.VMEM((_ROWS, d_model), bf16),
            pltpu.VMEM((2, d_model, _GRP * _DH), bf16),
            pltpu.VMEM((2, _DH, d_model), bf16),
            pltpu.VMEM((d_model, d_ff), bf16),
            pltpu.VMEM((d_model, d_ff), bf16),
            pltpu.VMEM((d_ff, d_model), bf16),
            pltpu.VMEM((2, _DH, win), bf16),
            pltpu.VMEM((2, _DH, win), bf16),
            pltpu.VMEM((2, _ROWS, _DH), bf16),
            pltpu.VMEM((_ROWS, win), f32),
            pltpu.VMEM((_ROWS, 128), f32),
            pltpu.VMEM((_ROWS, _DH), bf16),
            pltpu.VMEM((_ROWS, d_model), f32),
            dma((1,)), dma((2,)), dma((2,)), dma((2,)), dma((2,)),
            dma((40,)), dma((6,)),
        ],
        compiler_params=pltpu.CompilerParams(
            vmem_limit_bytes=48 * 1024 * 1024, disable_semaphore_checks=True,
            disable_bounds_checks=not BOUNDS),
    )(x2, k_t, v_t, A_wq, wo3, B_w1, B_w3, B_w2)
    return out.reshape(b, sq, d_model)
```

```python
import dataclasses
import functools

import jax
import jax.numpy as jnp
import jax.experimental.pallas as pl
import jax.experimental.pallas.tpu as pltpu

_HQ = 32
_DH = 192
_EPS = 1e-5
_ROWS = 8
_PAIR = 2 * _DH
_GRP = 4
_HI, _LO = 0, 1

_KV_W = (640, 640, 640, 640, 768, 768)
_KV_R = 32
_RB = 8
_LOOK = 24
_PRE = 2
_N_SL = 8
_W2_HI = 256
_W2_VPU = 256
_LAND = 15
_N_FFN_SEMS = 18


def _layernorm(x):
    m = jnp.mean(x, axis=-1, keepdims=True)
    c = x - m
    v = jnp.mean(c * c, axis=-1, keepdims=True)
    return c / jnp.sqrt(v + _EPS)


def _kernel(x_hbm, k_hbm, v_hbm, wq_hbm, wo_hbm, w1_hbm, w3_hbm, w2_hbm, o_ref,
            x_v, xn_v, wq_v, wo_v, w1_v, w3_v, w2_v, kbuf, vbuf, q_v, s_v, m_v, av_v, res_v,
            sem_x, sem_wq, sem_k, sem_v, sem_wo, sem_lo, sem_hi,
            *, win_start, win):
    f32, bf16 = jnp.float32, jnp.bfloat16
    d_model = x_v.shape[-1]
    d_ff = w1_v.shape[-1]
    n_rb = _DH // _KV_R
    n = n_rb * len(_KV_W)
    n_wq = d_model // _RB // _GRP
    n_wo = 2 * (_DH // _RB)
    wo_cols = ((0, 256), (256, d_model - 256))
    sl = win // _N_SL
    assert sum(_KV_W) == win and n_wq + n_wo <= 2 * n and _LOOK <= n and n_wq % 2 == 0
    assert d_ff == 4 * _PAIR and d_model == 5 * 128 and _GRP * _DH == d_ff // 2
    scale = _DH ** -0.5

    def ds(start, size, align):
        if isinstance(start, int):
            return pl.ds(start, size)
        return pl.ds(pl.multiple_of(start, align), size)

    def kv_copy(hbm, buf, sem, h, slot, t):
        rows = pl.ds((t % n_rb) * _KV_R, _KV_R)
        c, w = sum(_KV_W[:t // n_rb]), _KV_W[t // n_rb]
        return pltpu.make_async_copy(
            hbm.at[0, h, rows, pl.ds(win_start + c, w)],
            buf.at[slot, rows, pl.ds(c, w)], sem.at[slot])

    k_copy = functools.partial(kv_copy, k_hbm, kbuf, sem_k)
    v_copy = functools.partial(kv_copy, v_hbm, vbuf, sem_v)

    def wq_copy(grp, slot, r0, nrows):
        rows = ds(r0, nrows, _RB)
        return pltpu.make_async_copy(
            wq_hbm.at[rows, ds(grp * (_GRP * _DH), _GRP * _DH, 128)],
            wq_v.at[slot, rows, :], sem_wq.at[slot])

    def wo_copy(h, slot, b):
        rows, cols = pl.ds((b // 2) * _RB, _RB), pl.ds(*wo_cols[b % 2])
        return pltpu.make_async_copy(wo_hbm.at[h, rows, cols], wo_v.at[slot, rows, cols],
                                     sem_wo.at[slot])

    def block_copy(hbm, buf, r0, nrows, c0, ncols, sem):
        rows, cols = ds(r0, nrows, _RB), pl.ds(c0, ncols)
        return pltpu.make_async_copy(hbm.at[rows, cols], buf.at[rows, cols], sem)

    def wait_all(ref, sem):
        pltpu.make_async_copy(ref, ref, sem).wait()

    w1_hi = d_model // 2
    w3_lo = d_model - d_model // 4
    mxu_end = d_ff - _W2_VPU
    w2_groups, r = [], _W2_HI
    while r < mxu_end:
        w2_groups.append((r, 256 if mxu_end - r >= 512 else 128))
        r += w2_groups[-1][1]
    g_w3, g_w2 = 1, 5
    g_vpu = g_w2 + len(w2_groups)
    ffn_lo = ([(w1_hbm, w1_v, r, 16, 0, d_ff, 0) for r in range(w1_hi, d_model, 16)]
              + [(w3_hbm, w3_v, r, 16, 0, d_ff, g_w3 + r // 128) for r in range(0, w3_lo, 16)]
              + [(w2_hbm, w2_v, r, 32, 0, d_model, g_w2 + gi)
                 for gi, (r0, nr) in enumerate(w2_groups) for r in range(r0, r0 + nr, 32)]
              + [(w2_hbm, w2_v, r, 32, 0, d_model, g_vpu + i)
                 for i, r in enumerate(range(mxu_end, d_ff, 32))])
    ffn_hi = ([(w3_hbm, w3_v, r, _RB, c, d_ff // 2, 1)
               for r in range(w3_lo, d_model, _RB) for c in (0, d_ff // 2)]
              + [(w2_hbm, w2_v, r, _RB, 0, d_model, 2 + r // 128)
                 for r in range(0, _W2_HI, _RB)])
    assert ffn_lo[-1][6] + 1 == _N_FFN_SEMS and len(ffn_hi) <= len(ffn_lo)

    def ffn_lo_copy(i):
        return block_copy(*ffn_lo[i][:6], sem_lo.at[ffn_lo[i][6]])

    def ffn_hi_copy(i):
        return block_copy(*ffn_hi[i][:6], sem_hi.at[ffn_hi[i][6]])

    pieces = sorted([((i + 0.5) / n_wq, "q", i) for i in range(n_wq)]
                    + [((i + 0.5) / n_wo, "o", i) for i in range(n_wo)])
    piece_at = {(i * 2 * n) // len(pieces): p[1:] for i, p in enumerate(pieces)}
    n_a = sum(1 for t in piece_at if t < n)

    def start_hi(j, kind, b):
        slot, quarter = j & 1, j & (_GRP - 1)
        grp = (j >> 2) + 1
        if kind == "o":
            wo_copy(j, slot, b).start(priority=_HI)
        elif isinstance(j, int):
            wq_copy(grp, grp & 1, (quarter * n_wq + b) * _RB, _RB).start(priority=_HI)
        else:
            @pl.when(j < _HQ - _GRP)
            def _():
                wq_copy(grp, grp & 1, (quarter * n_wq + b) * _RB, _RB).start(priority=_HI)

            @pl.when(j >= _HQ - _GRP)
            def _():
                block_copy(w1_hbm, w1_v, (quarter * (n_wq // 2) + b // 2) * _RB, _RB,
                           (b % 2) * (d_ff // 2), d_ff // 2,
                           sem_hi.at[0]).start(priority=_HI)

    def qk_slice(slot, i, mx):
        cols = pl.ds(i * sl, sl)
        s = jnp.dot(q_v[slot], kbuf[slot, :, cols], preferred_element_type=f32) * scale
        s_v[:, cols] = s
        for c in range(sl // 128):
            mx = jnp.maximum(mx, s[:, c * 128:(c + 1) * 128])
        return mx

    def pv_slice(slot, i, carry):
        acc, den = carry
        cols = pl.ds(i * sl, sl)
        p = jnp.exp(s_v[:, cols] - jnp.concatenate([m_v[...]] * (sl // 128), axis=-1))
        for c in range(sl // 128):
            den = den + p[:, c * 128:(c + 1) * 128]
        acc = acc + jax.lax.dot_general(
            p.astype(bf16), vbuf[slot, :, cols], (((1,), (1,)), ((), ())),
            preferred_element_type=f32)
        return acc, den

    def pv_init():
        return jnp.zeros((_ROWS, _DH), f32), jnp.zeros((_ROWS, 128), f32)

    def pv_finish(acc, den):
        return (acc / jnp.sum(den, axis=-1, keepdims=True)).astype(bf16)

    def out_proj(slot, o):
        wait_all(wo_v.at[slot], sem_wo.at[slot])
        return jnp.dot(o, wo_v[slot], preferred_element_type=f32)

    def q_proj(slot, half):
        w = wq_v[slot, :, ds(half * _PAIR, _PAIR, 128)]
        q = jnp.dot(xn_v[...], w, preferred_element_type=f32).astype(bf16)
        q_v[0] = q[:, :_DH]
        q_v[1] = q[:, _DH:]

    x_copy = pltpu.make_async_copy(x_hbm, x_v, sem_x.at[0])
    seq0 = ([k_copy(0, 0, t) for t in range(n)]
            + [wq_copy(0, 0, r, 32) for r in range(0, d_model, 32)])
    n0 = len(seq0)
    seq0 += [v_copy(0, 0, t) for t in range(_LOOK)]
    hi0 = [p[1:] for p in pieces[:n_a]]
    hi0_at = {(i * n0) // (n_a - _PRE): p for i, p in enumerate(hi0[_PRE:])}
    x_copy.start(priority=_HI)
    for c in seq0[:_LOOK]:
        c.start(priority=_LO)
    for p in hi0[:_PRE]:
        start_hi(0, *p)
    for t in range(n0):
        seq0[t].wait()
        if t in hi0_at:
            start_hi(0, *hi0_at[t])
        seq0[t + _LOOK].start(priority=_LO)
        if t == 2:
            x_copy.wait()
            x = jnp.broadcast_to(x_v[...].astype(f32), (_ROWS, d_model))
            xn_v[...] = _layernorm(x).astype(bf16)
            res_v[...] = x
    q_proj(0, 0)

    gap = (n - 1) // _N_SL

    def phase(j, carry):
        slot = j & 1
        prev = 1 - slot
        gslot = (j >> 2) & 1
        quarter = j & (_GRP - 1)

        def tick(t):
            if t < n:
                k_copy(j, slot, t).wait()
            else:
                v_copy(j, slot, t - n).wait()
            if t in piece_at:
                start_hi(j, *piece_at[t])
            u = t + _LOOK
            if u < n:
                k_copy(j, slot, u).start(priority=_LO)
            elif u < 2 * n:
                v_copy(j, slot, u - n).start(priority=_LO)
            else:
                @pl.when(j + 1 < _HQ)
                def _():
                    k_copy(j + 1, prev, u - 2 * n).start(priority=_LO)

                @pl.when(j + 1 == _HQ)
                def _():
                    ffn_lo_copy(u - 2 * n).start(priority=_LO)

        @pl.when(j > 0)
        def _():
            pv = pv_init()
            for t in range(n):
                tick(t)
                if t % gap == 0 and t // gap < _N_SL:
                    pv = pv_slice(prev, t // gap, pv)
                if t == gap * _N_SL:
                    @pl.when(quarter == 0)
                    def _():
                        wait_all(wq_v.at[gslot], sem_wq.at[gslot])

                    @pl.when(slot == 0)
                    def _():
                        q_proj(gslot, quarter >> 1)
            av_v[...] = pv_finish(*pv)

        mx = jnp.full((_ROWS, 128), -jnp.inf, f32)
        for t in range(n):
            tick(n + t)
            if t % gap == 0 and t // gap < _N_SL:
                mx = qk_slice(slot, t // gap, mx)
            if t == gap * _N_SL:
                m_v[...] = jnp.broadcast_to(jnp.max(mx, axis=-1, keepdims=True), (_ROWS, 128))

                @pl.when(j > 0)
                def _():
                    res_v[...] += out_proj(prev, av_v[...])
        return carry

    jax.lax.fori_loop(0, _HQ, phase, 0)

    done = [0]

    def ticks_to(m):
        for i in range(done[0], m + 1):
            ffn_lo_copy(i).wait()
            if i < len(ffn_hi):
                ffn_hi_copy(i).start(priority=_HI)
            if i + _LOOK < len(ffn_lo):
                ffn_lo_copy(i + _LOOK).start(priority=_LO)
        done[0] = max(done[0], m + 1)

    def lo_done(group):
        return max(i for i, e in enumerate(ffn_lo) if e[6] == group)

    def hi_done(group):
        return max(i for i, e in enumerate(ffn_hi) if e[6] == group) + _LAND

    last = (_HQ - 1) & 1
    pv = pv_init()
    for i in range(_N_SL):
        ticks_to(i * 18 // _N_SL)
        pv = pv_slice(last, i, pv)
    ticks_to(18)
    hres = res_v[...] + out_proj(last, pv_finish(*pv))
    ticks_to(21)
    hn = _layernorm(hres).astype(bf16)

    t0 = max(lo_done(0), 23)
    ticks_to(t0)
    wait_all(w1_v.at[pl.ds(0, w1_hi), :], sem_hi.at[0])
    gates = []
    for s in range(4):
        gates.append(jnp.dot(hn, w1_v[:, s * _PAIR:(s + 1) * _PAIR],
                             preferred_element_type=f32))
        ticks_to(t0 + (5 * (s + 1)) // 2)
    gate = jnp.concatenate(gates, axis=-1)
    gate = gate * jax.nn.sigmoid(gate)

    def up_chunk(c):
        return jnp.dot(hn[:, c * 128:(c + 1) * 128], w3_v[c * 128:(c + 1) * 128, :],
                       preferred_element_type=f32)

    up = None
    for c in range(3):
        ticks_to(lo_done(g_w3 + c))
        up = up_chunk(c) if up is None else up + up_chunk(c)
    ticks_to(max(hi_done(1) + 1, lo_done(g_w3 + 3)))
    wait_all(w3_v.at[pl.ds(w3_lo, d_model - w3_lo), :], sem_hi.at[1])
    up = up + up_chunk(3) + up_chunk(4)
    act = (gate * up).astype(bf16)

    def down(r0, nr):
        return jnp.dot(act[:, r0:r0 + nr], w2_v[r0:r0 + nr, :], preferred_element_type=f32)

    act_col = jnp.concatenate(
        [jnp.broadcast_to(act[0:1, c:c + 128].astype(f32), (128, 128)).T
         for c in range(mxu_end, d_ff, 128)], axis=0)

    out = hres
    pending = list(range(_W2_HI // 128))
    for gi, (r0, nr) in enumerate(w2_groups):
        ticks_to(lo_done(g_w2 + gi))
        part = down(r0, nr)
        while pending and (hi_done(2 + pending[0]) <= lo_done(g_w2 + gi)
                           or gi == len(w2_groups) - 1):
            c = pending.pop(0)
            wait_all(w2_v.at[pl.ds(c * 128, 128), :], sem_hi.at[2 + c])
            part = part + down(c * 128, 128)
        out = out + part

    tail = jnp.zeros((8, d_model), f32)
    for i, r in enumerate(range(mxu_end, d_ff, 32)):
        ticks_to(lo_done(g_vpu + i))
        a = act_col[r - mxu_end:r - mxu_end + 32, :]
        prod = w2_v[r:r + 32, :].astype(f32) * jnp.concatenate([a] * (d_model // 128), axis=-1)
        for k in range(4):
            tail = tail + prod[k * 8:(k + 1) * 8, :]
    assert done[0] == len(ffn_lo)
    o_ref[...] = (out[0:1, :] + jnp.sum(tail, axis=0, keepdims=True)).astype(o_ref.dtype)


def _compiler_params():
    kwargs = dict(vmem_limit_bytes=48 * 1024 * 1024)
    if any(f.name == "disable_semaphore_checks" for f in dataclasses.fields(pltpu.CompilerParams)):
        kwargs["disable_semaphore_checks"] = True
    return pltpu.CompilerParams(**kwargs)


@jax.jit
def pallas_sequential_preLN__sliding_block_cached__glu_gated_swiglu__decode_kernel(
    A_x: jax.Array,
    A_k_cache: jax.Array,
    A_v_cache: jax.Array,
    A_wq: jax.Array,
    A_wo: jax.Array,
    B_x: jax.Array,
    B_w1: jax.Array,
    B_w3: jax.Array,
    B_w2: jax.Array,
):
    del B_x
    b, sq, d_model = A_x.shape
    hkv, sk = A_k_cache.shape[1], A_k_cache.shape[2]
    d_ff = B_w1.shape[1]
    assert b == 1 and sq == 1 and hkv == _HQ and A_k_cache.shape[3] == _DH
    win = min(4096, max(256, sk // 4))
    bf16, f32 = jnp.bfloat16, jnp.float32

    k_t = jnp.swapaxes(A_k_cache, 2, 3)
    v_t = jnp.swapaxes(A_v_cache, 2, 3)
    x2 = A_x.reshape(1, d_model)
    wo3 = A_wo.reshape(_HQ, _DH, d_model)

    dma = pltpu.SemaphoreType.DMA
    out = pl.pallas_call(
        functools.partial(_kernel, win_start=sk - win, win=win),
        out_shape=jax.ShapeDtypeStruct((1, d_model), A_x.dtype),
        in_specs=[pl.BlockSpec(memory_space=pl.ANY)] * 8,
        out_specs=pl.BlockSpec(memory_space=pltpu.VMEM),
        scratch_shapes=[
            pltpu.VMEM((1, d_model), bf16),
            pltpu.VMEM((_ROWS, d_model), bf16),
            pltpu.VMEM((2, d_model, _GRP * _DH), bf16),
            pltpu.VMEM((2, _DH, d_model), bf16),
            pltpu.VMEM((d_model, d_ff), bf16),
            pltpu.VMEM((d_model, d_ff), bf16),
            pltpu.VMEM((d_ff, d_model), bf16),
            pltpu.VMEM((2, _DH, win), bf16),
            pltpu.VMEM((2, _DH, win), bf16),
            pltpu.VMEM((2, _ROWS, _DH), bf16),
            pltpu.VMEM((_ROWS, win), f32),
            pltpu.VMEM((_ROWS, 128), f32),
            pltpu.VMEM((_ROWS, _DH), bf16),
            pltpu.VMEM((_ROWS, d_model), f32),
            dma((1,)), dma((2,)), dma((2,)), dma((2,)), dma((2,)),
            dma((_N_FFN_SEMS,)), dma((2 + _W2_HI // 128,)),
        ],
        compiler_params=_compiler_params(),
    )(x2, k_t, v_t, A_wq, wo3, B_w1, B_w3, B_w2)
    return out.reshape(b, sq, d_model)
```

```python
import dataclasses
import functools

import jax
import jax.numpy as jnp
import numpy as np
import jax.experimental.pallas as pl
import jax.experimental.pallas.tpu as pltpu

_HQ = 32
_DH = 192
_EPS = float(np.asarray(1e-5, dtype=jnp.bfloat16))
_SCALE = float(np.asarray(_DH ** -0.5, dtype=jnp.bfloat16))
_ROWS = 8
_PAIR = 2 * _DH
_GRP = 4
_HI, _LO = 0, 1

_KV_W = (384, 768, 640, 768, 768, 768)
_KV_R = 32
_RB = 8
_LOOK = 24
_PRE = 2
_N_SL = 8
_W2_HI = 256
_W2_VPU = 256
_LAND = 15
_N_FFN_SEMS = 18


def _rnd(x):
    return x.astype(jnp.bfloat16).astype(jnp.float32)


def _layernorm(x):
    m = jnp.mean(x, axis=-1, keepdims=True)
    c = x - m
    v = jnp.mean(c * c, axis=-1, keepdims=True)
    return _rnd(x - _rnd(m)) / _rnd(jnp.sqrt(_rnd(_rnd(v) + _EPS)))


def _kernel(x_hbm, k_hbm, v_hbm, wq_hbm, wo_hbm, w1_hbm, w3_hbm, w2_hbm, o_ref,
            x_v, xn_v, wq_v, wo_v, w1_v, w3_v, w2_v, kbuf, vbuf, q_v, s_v, m_v, av_v, res_v,
            sem_x, sem_wq, sem_k, sem_v, sem_wo, sem_lo, sem_hi,
            *, win_start, win):
    f32, bf16 = jnp.float32, jnp.bfloat16
    d_model = x_v.shape[-1]
    d_ff = w1_v.shape[-1]
    n_rb = _DH // _KV_R
    n = n_rb * len(_KV_W)
    n_wq = d_model // _RB // _GRP
    n_wo = 2 * (_DH // _RB)
    wo_cols = ((0, 256), (256, d_model - 256))
    sl = win // _N_SL
    assert sum(_KV_W) == win and n_wq + n_wo <= 2 * n and _LOOK <= n and n_wq % 2 == 0
    assert d_ff == 4 * _PAIR and d_model == 5 * 128 and _GRP * _DH == d_ff // 2

    def ds(start, size, align):
        if isinstance(start, int):
            return pl.ds(start, size)
        return pl.ds(pl.multiple_of(start, align), size)

    def kv_copy(hbm, buf, sem, h, slot, t):
        rows = pl.ds((t % n_rb) * _KV_R, _KV_R)
        c, w = sum(_KV_W[:t // n_rb]), _KV_W[t // n_rb]
        return pltpu.make_async_copy(
            hbm.at[0, h, rows, pl.ds(win_start + c, w)],
            buf.at[slot, rows, pl.ds(c, w)], sem.at[slot])

    k_copy = functools.partial(kv_copy, k_hbm, kbuf, sem_k)
    v_copy = functools.partial(kv_copy, v_hbm, vbuf, sem_v)

    def wq_copy(grp, slot, r0, nrows):
        rows = ds(r0, nrows, _RB)
        return pltpu.make_async_copy(
            wq_hbm.at[rows, ds(grp * (_GRP * _DH), _GRP * _DH, 128)],
            wq_v.at[slot, rows, :], sem_wq.at[slot])

    def wo_copy(h, slot, b):
        rows, cols = pl.ds((b // 2) * _RB, _RB), pl.ds(*wo_cols[b % 2])
        return pltpu.make_async_copy(wo_hbm.at[h, rows, cols], wo_v.at[slot, rows, cols],
                                     sem_wo.at[slot])

    def block_copy(hbm, buf, r0, nrows, c0, ncols, sem):
        rows, cols = ds(r0, nrows, _RB), pl.ds(c0, ncols)
        return pltpu.make_async_copy(hbm.at[rows, cols], buf.at[rows, cols], sem)

    def wait_all(ref, sem):
        pltpu.make_async_copy(ref, ref, sem).wait()

    w1_hi = d_model // 2
    w3_lo = d_model - d_model // 4
    mxu_end = d_ff - _W2_VPU
    w2_groups, r = [], _W2_HI
    while r < mxu_end:
        w2_groups.append((r, 256 if mxu_end - r >= 512 else 128))
        r += w2_groups[-1][1]
    g_w3, g_w2 = 1, 5
    g_vpu = g_w2 + len(w2_groups)
    ffn_lo = ([(w1_hbm, w1_v, r, 16, 0, d_ff, 0) for r in range(w1_hi, d_model, 16)]
              + [(w3_hbm, w3_v, r, 16, 0, d_ff, g_w3 + r // 128) for r in range(0, w3_lo, 16)]
              + [(w2_hbm, w2_v, r, 32, 0, d_model, g_w2 + gi)
                 for gi, (r0, nr) in enumerate(w2_groups) for r in range(r0, r0 + nr, 32)]
              + [(w2_hbm, w2_v, r, 32, 0, d_model, g_vpu + i)
                 for i, r in enumerate(range(mxu_end, d_ff, 32))])
    ffn_hi = ([(w3_hbm, w3_v, r, _RB, c, d_ff // 2, 1)
               for r in range(w3_lo, d_model, _RB) for c in (0, d_ff // 2)]
              + [(w2_hbm, w2_v, r, _RB, 0, d_model, 2 + r // 128)
                 for r in range(0, _W2_HI, _RB)])
    assert ffn_lo[-1][6] + 1 == _N_FFN_SEMS and len(ffn_hi) <= len(ffn_lo)

    def ffn_lo_copy(i):
        return block_copy(*ffn_lo[i][:6], sem_lo.at[ffn_lo[i][6]])

    def ffn_hi_copy(i):
        return block_copy(*ffn_hi[i][:6], sem_hi.at[ffn_hi[i][6]])

    pieces = sorted([((i + 0.5) / n_wq, "q", i) for i in range(n_wq)]
                    + [((i + 0.5) / n_wo, "o", i) for i in range(n_wo)])
    piece_at = {(i * 2 * n) // len(pieces): p[1:] for i, p in enumerate(pieces)}
    n_a = sum(1 for t in piece_at if t < n)

    def start_hi(j, kind, b):
        slot, quarter = j & 1, j & (_GRP - 1)
        grp = (j >> 2) + 1
        if kind == "o":
            wo_copy(j, slot, b).start(priority=_HI)
        elif isinstance(j, int):
            wq_copy(grp, grp & 1, (quarter * n_wq + b) * _RB, _RB).start(priority=_HI)
        else:
            @pl.when(j < _HQ - _GRP)
            def _():
                wq_copy(grp, grp & 1, (quarter * n_wq + b) * _RB, _RB).start(priority=_HI)

            @pl.when(j >= _HQ - _GRP)
            def _():
                block_copy(w1_hbm, w1_v, (quarter * (n_wq // 2) + b // 2) * _RB, _RB,
                           (b % 2) * (d_ff // 2), d_ff // 2,
                           sem_hi.at[0]).start(priority=_HI)

    def qk_slice(slot, i, mx):
        cols = pl.ds(i * sl, sl)
        s = jnp.dot(q_v[slot], kbuf[slot, :, cols], preferred_element_type=f32)
        s = _rnd(_rnd(s) * _SCALE)
        s_v[:, cols] = s
        for c in range(sl // 128):
            mx = jnp.maximum(mx, s[:, c * 128:(c + 1) * 128])
        return mx

    def pv_slice(slot, i, carry):
        acc, den = carry
        cols = pl.ds(i * sl, sl)
        p = jnp.exp(s_v[:, cols] - jnp.concatenate([m_v[...]] * (sl // 128), axis=-1))
        for c in range(sl // 128):
            den = den + p[:, c * 128:(c + 1) * 128]
        acc = acc + jax.lax.dot_general(
            p.astype(bf16), vbuf[slot, :, cols], (((1,), (1,)), ((), ())),
            preferred_element_type=f32)
        return acc, den

    def pv_init():
        return jnp.zeros((_ROWS, _DH), f32), jnp.zeros((_ROWS, 128), f32)

    def pv_finish(acc, den):
        return (acc / jnp.sum(den, axis=-1, keepdims=True)).astype(bf16)

    def out_proj(slot, o):
        wait_all(wo_v.at[slot], sem_wo.at[slot])
        return jnp.dot(o, wo_v[slot], preferred_element_type=f32)

    def q_proj(slot, half):
        w = wq_v[slot, :, ds(half * _PAIR, _PAIR, 128)]
        q = jnp.dot(xn_v[...], w, preferred_element_type=f32).astype(bf16)
        q_v[0] = q[:, :_DH]
        q_v[1] = q[:, _DH:]

    x_copy = pltpu.make_async_copy(x_hbm, x_v, sem_x.at[0])
    seq0 = ([k_copy(0, 0, t) for t in range(n)]
            + [wq_copy(0, 0, r, 32) for r in range(0, d_model, 32)])
    n0 = len(seq0)
    seq0 += [v_copy(0, 0, t) for t in range(_LOOK)]
    hi0 = [p[1:] for p in pieces[:n_a]]
    hi0_at = {(i * n0) // (n_a - _PRE): p for i, p in enumerate(hi0[_PRE:])}
    x_copy.start(priority=_HI)
    for c in seq0[:_LOOK]:
        c.start(priority=_LO)
    for p in hi0[:_PRE]:
        start_hi(0, *p)
    for t in range(n0):
        seq0[t].wait()
        if t in hi0_at:
            start_hi(0, *hi0_at[t])
        seq0[t + _LOOK].start(priority=_LO)
        if t == 2:
            x_copy.wait()
            x = jnp.broadcast_to(x_v[...].astype(f32), (_ROWS, d_model))
            xn_v[...] = _layernorm(x).astype(bf16)
            res_v[...] = jnp.zeros_like(x)
    q_proj(0, 0)

    gap = (n - 1) // _N_SL

    def phase(j, carry):
        slot = j & 1
        prev = 1 - slot
        gslot = (j >> 2) & 1
        quarter = j & (_GRP - 1)

        def tick(t):
            if t < n:
                k_copy(j, slot, t).wait()
            else:
                v_copy(j, slot, t - n).wait()
            if t in piece_at:
                start_hi(j, *piece_at[t])
            u = t + _LOOK
            if u < n:
                k_copy(j, slot, u).start(priority=_LO)
            elif u < 2 * n:
                v_copy(j, slot, u - n).start(priority=_LO)
            else:
                @pl.when(j + 1 < _HQ)
                def _():
                    k_copy(j + 1, prev, u - 2 * n).start(priority=_LO)

                @pl.when(j + 1 == _HQ)
                def _():
                    ffn_lo_copy(u - 2 * n).start(priority=_LO)

        @pl.when(j > 0)
        def _():
            pv = pv_init()
            for t in range(n):
                tick(t)
                if t % gap == 0 and t // gap < _N_SL:
                    pv = pv_slice(prev, t // gap, pv)
                if t == gap * _N_SL:
                    @pl.when(quarter == 0)
                    def _():
                        wait_all(wq_v.at[gslot], sem_wq.at[gslot])

                    @pl.when(slot == 0)
                    def _():
                        q_proj(gslot, quarter >> 1)
            av_v[...] = pv_finish(*pv)

        mx = jnp.full((_ROWS, 128), -jnp.inf, f32)
        for t in range(n):
            tick(n + t)
            if t % gap == 0 and t // gap < _N_SL:
                mx = qk_slice(slot, t // gap, mx)
            if t == gap * _N_SL:
                m_v[...] = jnp.broadcast_to(jnp.max(mx, axis=-1, keepdims=True), (_ROWS, 128))

                @pl.when(j > 0)
                def _():
                    res_v[...] += out_proj(prev, av_v[...])
        return carry

    jax.lax.fori_loop(0, _HQ, phase, 0)

    done = [0]

    def ticks_to(m):
        for i in range(done[0], m + 1):
            ffn_lo_copy(i).wait()
            if i < len(ffn_hi):
                ffn_hi_copy(i).start(priority=_HI)
            if i + _LOOK < len(ffn_lo):
                ffn_lo_copy(i + _LOOK).start(priority=_LO)
        done[0] = max(done[0], m + 1)

    def lo_done(group):
        return max(i for i, e in enumerate(ffn_lo) if e[6] == group)

    def hi_done(group):
        return max(i for i, e in enumerate(ffn_hi) if e[6] == group) + _LAND

    last = (_HQ - 1) & 1
    pv = pv_init()
    for i in range(_N_SL):
        ticks_to(i * 18 // _N_SL)
        pv = pv_slice(last, i, pv)
    ticks_to(18)
    hres = _rnd(x + _rnd(res_v[...] + out_proj(last, pv_finish(*pv))))
    ticks_to(21)
    hn = _layernorm(hres).astype(bf16)

    t0 = max(lo_done(0), 23)
    ticks_to(t0)
    wait_all(w1_v.at[pl.ds(0, w1_hi), :], sem_hi.at[0])
    gates = []
    for s in range(4):
        gates.append(jnp.dot(hn, w1_v[:, s * _PAIR:(s + 1) * _PAIR],
                             preferred_element_type=f32))
        ticks_to(t0 + (5 * (s + 1)) // 2)
    gate = _rnd(jnp.concatenate(gates, axis=-1))
    gate = _rnd(gate * jax.nn.sigmoid(gate))

    def up_chunk(c):
        return jnp.dot(hn[:, c * 128:(c + 1) * 128], w3_v[c * 128:(c + 1) * 128, :],
                       preferred_element_type=f32)

    up = None
    for c in range(3):
        ticks_to(lo_done(g_w3 + c))
        up = up_chunk(c) if up is None else up + up_chunk(c)
    ticks_to(max(hi_done(1) + 1, lo_done(g_w3 + 3)))
    wait_all(w3_v.at[pl.ds(w3_lo, d_model - w3_lo), :], sem_hi.at[1])
    up = up + up_chunk(3) + up_chunk(4)
    act = (gate * _rnd(up)).astype(bf16)

    def down(r0, nr):
        return jnp.dot(act[:, r0:r0 + nr], w2_v[r0:r0 + nr, :], preferred_element_type=f32)

    act_col = jnp.concatenate(
        [jnp.broadcast_to(act[0:1, c:c + 128].astype(f32), (128, 128)).T
         for c in range(mxu_end, d_ff, 128)], axis=0)

    out = jnp.zeros_like(hres)
    pending = list(range(_W2_HI // 128))
    for gi, (r0, nr) in enumerate(w2_groups):
        ticks_to(lo_done(g_w2 + gi))
        part = down(r0, nr)
        while pending and (hi_done(2 + pending[0]) <= lo_done(g_w2 + gi)
                           or gi == len(w2_groups) - 1):
            c = pending.pop(0)
            wait_all(w2_v.at[pl.ds(c * 128, 128), :], sem_hi.at[2 + c])
            part = part + down(c * 128, 128)
        out = out + part

    tail = jnp.zeros((8, d_model), f32)
    for i, r in enumerate(range(mxu_end, d_ff, 32)):
        ticks_to(lo_done(g_vpu + i))
        a = act_col[r - mxu_end:r - mxu_end + 32, :]
        prod = w2_v[r:r + 32, :].astype(f32) * jnp.concatenate([a] * (d_model // 128), axis=-1)
        for k in range(4):
            tail = tail + prod[k * 8:(k + 1) * 8, :]
    assert done[0] == len(ffn_lo)
    ffn = out[0:1, :] + jnp.sum(tail, axis=0, keepdims=True)
    o_ref[...] = (hres[0:1, :] + _rnd(ffn)).astype(o_ref.dtype)


def _compiler_params():
    kwargs = dict(vmem_limit_bytes=48 * 1024 * 1024)
    if any(f.name == "disable_semaphore_checks" for f in dataclasses.fields(pltpu.CompilerParams)):
        kwargs["disable_semaphore_checks"] = True
    return pltpu.CompilerParams(**kwargs)


@jax.jit
def pallas_sequential_preLN__sliding_block_cached__glu_gated_swiglu__decode_kernel(
    A_x: jax.Array,
    A_k_cache: jax.Array,
    A_v_cache: jax.Array,
    A_wq: jax.Array,
    A_wo: jax.Array,
    B_x: jax.Array,
    B_w1: jax.Array,
    B_w3: jax.Array,
    B_w2: jax.Array,
):
    del B_x
    b, sq, d_model = A_x.shape
    hkv, sk = A_k_cache.shape[1], A_k_cache.shape[2]
    d_ff = B_w1.shape[1]
    assert b == 1 and sq == 1 and hkv == _HQ and A_k_cache.shape[3] == _DH
    win = min(4096, max(256, sk // 4))
    bf16, f32 = jnp.bfloat16, jnp.float32

    k_t = jnp.swapaxes(A_k_cache, 2, 3)
    v_t = jnp.swapaxes(A_v_cache, 2, 3)
    x2 = A_x.reshape(1, d_model)
    wo3 = A_wo.reshape(_HQ, _DH, d_model)

    dma = pltpu.SemaphoreType.DMA
    out = pl.pallas_call(
        functools.partial(_kernel, win_start=sk - win, win=win),
        out_shape=jax.ShapeDtypeStruct((1, d_model), A_x.dtype),
        in_specs=[pl.BlockSpec(memory_space=pl.ANY)] * 8,
        out_specs=pl.BlockSpec(memory_space=pltpu.VMEM),
        scratch_shapes=[
            pltpu.VMEM((1, d_model), bf16),
            pltpu.VMEM((_ROWS, d_model), bf16),
            pltpu.VMEM((2, d_model, _GRP * _DH), bf16),
            pltpu.VMEM((2, _DH, d_model), bf16),
            pltpu.VMEM((d_model, d_ff), bf16),
            pltpu.VMEM((d_model, d_ff), bf16),
            pltpu.VMEM((d_ff, d_model), bf16),
            pltpu.VMEM((2, _DH, win), bf16),
            pltpu.VMEM((2, _DH, win), bf16),
            pltpu.VMEM((2, _ROWS, _DH), bf16),
            pltpu.VMEM((_ROWS, win), f32),
            pltpu.VMEM((_ROWS, 128), f32),
            pltpu.VMEM((_ROWS, _DH), bf16),
            pltpu.VMEM((_ROWS, d_model), f32),
            dma((1,)), dma((2,)), dma((2,)), dma((2,)), dma((2,)),
            dma((_N_FFN_SEMS,)), dma((2 + _W2_HI // 128,)),
        ],
        compiler_params=_compiler_params(),
    )(x2, k_t, v_t, A_wq, wo3, B_w1, B_w3, B_w2)
    return out.reshape(b, sq, d_model)
```

```python
import dataclasses
import functools

import jax
import jax.numpy as jnp
import numpy as np
import jax.experimental.pallas as pl
import jax.experimental.pallas.tpu as pltpu

_HQ = 32
_DH = 192
_EPS = float(np.asarray(1e-5, dtype=jnp.bfloat16))
_SCALE = float(np.asarray(_DH ** -0.5, dtype=jnp.bfloat16))
_ROWS = 8
_PAIR = 2 * _DH
_GRP = 4
_HI, _LO = 0, 1

_KV_W = (384, 768, 640, 768, 768, 768)
_KV_R = 32
_RB = 8
_LOOK = 24
_PRE = 2
_N_SL = 8
_W2_HI = 256
_W2_VPU = 256
_LAND = 15
_N_FFN_SEMS = 18


def _rnd(x):
    return x.astype(jnp.bfloat16).astype(jnp.float32)


def _layernorm(x):
    m = jnp.mean(x, axis=-1, keepdims=True)
    c = x - m
    v = jnp.mean(c * c, axis=-1, keepdims=True)
    return _rnd(x - _rnd(m)) / _rnd(jnp.sqrt(_rnd(_rnd(v) + _EPS)))


def _kernel(x_hbm, k_hbm, v_hbm, wq_hbm, wo_hbm, w1_hbm, w3_hbm, w2_hbm, o_ref,
            x_v, xn_v, wq_v, wo_v, w1_v, w3_v, w2_v, kbuf, vbuf, q_v, s_v, m_v, av_v, res_v,
            sem_x, sem_wq, sem_k, sem_v, sem_wo, sem_lo, sem_hi,
            *, win_start, win):
    f32, bf16 = jnp.float32, jnp.bfloat16
    d_model = x_v.shape[-1]
    d_ff = w1_v.shape[-1]
    n_rb = _DH // _KV_R
    n = n_rb * len(_KV_W)
    n_wq = d_model // _RB // _GRP
    n_wo = 2 * (_DH // _RB)
    wo_cols = ((0, 256), (256, d_model - 256))
    sl = win // _N_SL
    assert sum(_KV_W) == win and n_wq + n_wo <= 2 * n and _LOOK <= n and n_wq % 2 == 0
    assert d_ff == 4 * _PAIR and d_model == 5 * 128 and _GRP * _DH == d_ff // 2

    def ds(start, size, align):
        if isinstance(start, int):
            return pl.ds(start, size)
        return pl.ds(pl.multiple_of(start, align), size)

    def kv_copy(hbm, buf, sem, h, slot, t):
        rows = pl.ds((t % n_rb) * _KV_R, _KV_R)
        c, w = sum(_KV_W[:t // n_rb]), _KV_W[t // n_rb]
        return pltpu.make_async_copy(
            hbm.at[0, h, rows, pl.ds(win_start + c, w)],
            buf.at[slot, rows, pl.ds(c, w)], sem.at[slot])

    k_copy = functools.partial(kv_copy, k_hbm, kbuf, sem_k)
    v_copy = functools.partial(kv_copy, v_hbm, vbuf, sem_v)

    def wq_copy(grp, slot, r0, nrows):
        rows = ds(r0, nrows, _RB)
        return pltpu.make_async_copy(
            wq_hbm.at[rows, ds(grp * (_GRP * _DH), _GRP * _DH, 128)],
            wq_v.at[slot, rows, :], sem_wq.at[slot])

    def wo_copy(h, slot, b):
        rows, cols = pl.ds((b // 2) * _RB, _RB), pl.ds(*wo_cols[b % 2])
        return pltpu.make_async_copy(wo_hbm.at[h, rows, cols], wo_v.at[slot, rows, cols],
                                     sem_wo.at[slot])

    def block_copy(hbm, buf, r0, nrows, c0, ncols, sem):
        rows, cols = ds(r0, nrows, _RB), pl.ds(c0, ncols)
        return pltpu.make_async_copy(hbm.at[rows, cols], buf.at[rows, cols], sem)

    def wait_all(ref, sem):
        pltpu.make_async_copy(ref, ref, sem).wait()

    w1_hi = d_model // 2
    w3_lo = d_model - d_model // 4
    mxu_end = d_ff - _W2_VPU
    w2_groups, r = [], _W2_HI
    while r < mxu_end:
        w2_groups.append((r, 256 if mxu_end - r >= 512 else 128))
        r += w2_groups[-1][1]
    g_w3, g_w2 = 1, 5
    g_vpu = g_w2 + len(w2_groups)
    lo1 = [(w1_hbm, w1_v, r, 16, 0, d_ff, 0) for r in range(w1_hi, d_model, 16)]
    lo3 = [(w3_hbm, w3_v, r, 16, 0, d_ff, g_w3 + r // 128) for r in range(0, w3_lo, 16)]
    mixed = sorted([(0.6 * (i + 0.5) / len(lo1), 0, i) for i in range(len(lo1))]
                   + [((i + 0.5) / len(lo3), 1, i) for i in range(len(lo3))])
    ffn_lo = ([(lo1, lo3)[which][i] for _, which, i in mixed]
              + [(w2_hbm, w2_v, r, 32, 0, d_model, g_w2 + gi)
                 for gi, (r0, nr) in enumerate(w2_groups) for r in range(r0, r0 + nr, 32)]
              + [(w2_hbm, w2_v, r, 32, 0, d_model, g_vpu + i)
                 for i, r in enumerate(range(mxu_end, d_ff, 32))])
    ffn_hi = ([(w3_hbm, w3_v, r, _RB, c, d_ff // 2, 1)
               for r in range(w3_lo, d_model, _RB) for c in (0, d_ff // 2)]
              + [(w2_hbm, w2_v, r, _RB, 0, d_model, 2 + r // 128)
                 for r in range(0, _W2_HI, _RB)])
    assert ffn_lo[-1][6] + 1 == _N_FFN_SEMS and len(ffn_hi) <= len(ffn_lo)

    def ffn_lo_copy(i):
        return block_copy(*ffn_lo[i][:6], sem_lo.at[ffn_lo[i][6]])

    def ffn_hi_copy(i):
        return block_copy(*ffn_hi[i][:6], sem_hi.at[ffn_hi[i][6]])

    pieces = sorted([((i + 0.5) / n_wq, "q", i) for i in range(n_wq)]
                    + [((i + 0.5) / n_wo, "o", i) for i in range(n_wo)])
    piece_at = {(i * 2 * n) // len(pieces): p[1:] for i, p in enumerate(pieces)}
    n_a = sum(1 for t in piece_at if t < n)

    def start_hi(j, kind, b):
        slot, quarter = j & 1, j & (_GRP - 1)
        grp = (j >> 2) + 1
        if kind == "o":
            wo_copy(j, slot, b).start(priority=_HI)
        elif isinstance(j, int):
            wq_copy(grp, grp & 1, (quarter * n_wq + b) * _RB, _RB).start(priority=_HI)
        else:
            @pl.when(j < _HQ - _GRP)
            def _():
                wq_copy(grp, grp & 1, (quarter * n_wq + b) * _RB, _RB).start(priority=_HI)

            @pl.when(j >= _HQ - _GRP)
            def _():
                block_copy(w1_hbm, w1_v, (quarter * (n_wq // 2) + b // 2) * _RB, _RB,
                           (b % 2) * (d_ff // 2), d_ff // 2,
                           sem_hi.at[0]).start(priority=_HI)

    def qk_slice(slot, i, mx):
        cols = pl.ds(i * sl, sl)
        s = jnp.dot(q_v[slot], kbuf[slot, :, cols], preferred_element_type=f32)
        s = _rnd(_rnd(s) * _SCALE)
        s_v[:, cols] = s
        for c in range(sl // 128):
            mx = jnp.maximum(mx, s[:, c * 128:(c + 1) * 128])
        return mx

    def pv_slice(slot, i, carry):
        acc, den = carry
        cols = pl.ds(i * sl, sl)
        p = jnp.exp(s_v[:, cols] - jnp.concatenate([m_v[...]] * (sl // 128), axis=-1))
        for c in range(sl // 128):
            den = den + p[:, c * 128:(c + 1) * 128]
        acc = acc + jax.lax.dot_general(
            p.astype(bf16), vbuf[slot, :, cols], (((1,), (1,)), ((), ())),
            preferred_element_type=f32)
        return acc, den

    def pv_init():
        return jnp.zeros((_ROWS, _DH), f32), jnp.zeros((_ROWS, 128), f32)

    def pv_finish(acc, den):
        return (acc / jnp.sum(den, axis=-1, keepdims=True)).astype(bf16)

    def out_proj(slot, o):
        wait_all(wo_v.at[slot], sem_wo.at[slot])
        return jnp.dot(o, wo_v[slot], preferred_element_type=f32)

    def q_proj(slot, half):
        w = wq_v[slot, :, ds(half * _PAIR, _PAIR, 128)]
        q = jnp.dot(xn_v[...], w, preferred_element_type=f32).astype(bf16)
        q_v[0] = q[:, :_DH]
        q_v[1] = q[:, _DH:]

    x_copy = pltpu.make_async_copy(x_hbm, x_v, sem_x.at[0])
    seq0 = ([k_copy(0, 0, t) for t in range(n)]
            + [wq_copy(0, 0, r, 32) for r in range(0, d_model, 32)])
    n0 = len(seq0)
    seq0 += [v_copy(0, 0, t) for t in range(_LOOK)]
    hi0 = [p[1:] for p in pieces[:n_a]]
    hi0_at = {(i * n0) // (n_a - _PRE): p for i, p in enumerate(hi0[_PRE:])}
    x_copy.start(priority=_HI)
    for c in seq0[:_LOOK]:
        c.start(priority=_LO)
    for p in hi0[:_PRE]:
        start_hi(0, *p)
    for t in range(n0):
        seq0[t].wait()
        if t in hi0_at:
            start_hi(0, *hi0_at[t])
        seq0[t + _LOOK].start(priority=_LO)
        if t == 2:
            x_copy.wait()
            x = jnp.broadcast_to(x_v[...].astype(f32), (_ROWS, d_model))
            xn_v[...] = _layernorm(x).astype(bf16)
            res_v[...] = jnp.zeros_like(x)
    q_proj(0, 0)

    gap = (n - 1) // _N_SL

    def phase(j, carry):
        slot = j & 1
        prev = 1 - slot
        gslot = (j >> 2) & 1
        quarter = j & (_GRP - 1)

        def tick(t):
            if t < n:
                k_copy(j, slot, t).wait()
            else:
                v_copy(j, slot, t - n).wait()
            if t in piece_at:
                start_hi(j, *piece_at[t])
            u = t + _LOOK
            if u < n:
                k_copy(j, slot, u).start(priority=_LO)
            elif u < 2 * n:
                v_copy(j, slot, u - n).start(priority=_LO)
            else:
                @pl.when(j + 1 < _HQ)
                def _():
                    k_copy(j + 1, prev, u - 2 * n).start(priority=_LO)

                @pl.when(j + 1 == _HQ)
                def _():
                    ffn_lo_copy(u - 2 * n).start(priority=_LO)

        @pl.when(j > 0)
        def _():
            pv = pv_init()
            for t in range(n):
                tick(t)
                if t % gap == 0 and t // gap < _N_SL:
                    pv = pv_slice(prev, t // gap, pv)
                if t == gap * _N_SL:
                    @pl.when(quarter == 0)
                    def _():
                        wait_all(wq_v.at[gslot], sem_wq.at[gslot])

                    @pl.when(slot == 0)
                    def _():
                        q_proj(gslot, quarter >> 1)
            av_v[...] = pv_finish(*pv)

        mx = jnp.full((_ROWS, 128), -jnp.inf, f32)
        for t in range(n):
            tick(n + t)
            if t % gap == 0 and t // gap < _N_SL:
                mx = qk_slice(slot, t // gap, mx)
            if t == gap * _N_SL:
                m_v[...] = jnp.broadcast_to(jnp.max(mx, axis=-1, keepdims=True), (_ROWS, 128))

                @pl.when(j > 0)
                def _():
                    res_v[...] += out_proj(prev, av_v[...])
        return carry

    jax.lax.fori_loop(0, _HQ, phase, 0)

    done = [0]

    def ticks_to(m):
        for i in range(done[0], m + 1):
            ffn_lo_copy(i).wait()
            if i < len(ffn_hi):
                ffn_hi_copy(i).start(priority=_HI)
            if i + _LOOK < len(ffn_lo):
                ffn_lo_copy(i + _LOOK).start(priority=_LO)
        done[0] = max(done[0], m + 1)

    def lo_done(group):
        return max(i for i, e in enumerate(ffn_lo) if e[6] == group)

    def hi_done(group):
        return max(i for i, e in enumerate(ffn_hi) if e[6] == group) + _LAND

    last = (_HQ - 1) & 1
    pv = pv_init()
    for i in range(_N_SL):
        ticks_to(i * 18 // _N_SL)
        pv = pv_slice(last, i, pv)
    ticks_to(18)
    hres = _rnd(x + _rnd(res_v[...] + out_proj(last, pv_finish(*pv))))
    ticks_to(21)
    hn = _layernorm(hres).astype(bf16)

    t0 = max(lo_done(0), 23)
    ticks_to(t0)
    wait_all(w1_v.at[pl.ds(0, w1_hi), :], sem_hi.at[0])
    gates = []
    for s in range(4):
        gates.append(jnp.dot(hn, w1_v[:, s * _PAIR:(s + 1) * _PAIR],
                             preferred_element_type=f32))
        ticks_to(t0 + (5 * (s + 1)) // 2)
    gate = _rnd(jnp.concatenate(gates, axis=-1))
    gate = _rnd(gate * jax.nn.sigmoid(gate))

    def up_chunk(c):
        return jnp.dot(hn[:, c * 128:(c + 1) * 128], w3_v[c * 128:(c + 1) * 128, :],
                       preferred_element_type=f32)

    up = None
    for c in range(3):
        ticks_to(lo_done(g_w3 + c))
        up = up_chunk(c) if up is None else up + up_chunk(c)
    ticks_to(max(hi_done(1) + 1, lo_done(g_w3 + 3)))
    wait_all(w3_v.at[pl.ds(w3_lo, d_model - w3_lo), :], sem_hi.at[1])
    up = up + up_chunk(3) + up_chunk(4)
    act = (gate * _rnd(up)).astype(bf16)

    def down(r0, nr):
        return jnp.dot(act[:, r0:r0 + nr], w2_v[r0:r0 + nr, :], preferred_element_type=f32)

    act_col = jnp.concatenate(
        [jnp.broadcast_to(act[0:1, c:c + 128].astype(f32), (128, 128)).T
         for c in range(mxu_end, d_ff, 128)], axis=0)

    out = jnp.zeros_like(hres)
    pending = list(range(_W2_HI // 128))
    for gi, (r0, nr) in enumerate(w2_groups):
        ticks_to(lo_done(g_w2 + gi))
        part = down(r0, nr)
        while pending and (hi_done(2 + pending[0]) <= lo_done(g_w2 + gi)
                           or gi == len(w2_groups) - 1):
            c = pending.pop(0)
            wait_all(w2_v.at[pl.ds(c * 128, 128), :], sem_hi.at[2 + c])
            part = part + down(c * 128, 128)
        out = out + part

    tail = jnp.zeros((8, d_model), f32)
    for i, r in enumerate(range(mxu_end, d_ff, 32)):
        ticks_to(lo_done(g_vpu + i))
        a = act_col[r - mxu_end:r - mxu_end + 32, :]
        prod = w2_v[r:r + 32, :].astype(f32) * jnp.concatenate([a] * (d_model // 128), axis=-1)
        for k in range(4):
            tail = tail + prod[k * 8:(k + 1) * 8, :]
    assert done[0] == len(ffn_lo)
    ffn = out[0:1, :] + jnp.sum(tail, axis=0, keepdims=True)
    o_ref[...] = (hres[0:1, :] + _rnd(ffn)).astype(o_ref.dtype)


def _compiler_params():
    kwargs = dict(vmem_limit_bytes=48 * 1024 * 1024)
    if any(f.name == "disable_semaphore_checks" for f in dataclasses.fields(pltpu.CompilerParams)):
        kwargs["disable_semaphore_checks"] = True
    return pltpu.CompilerParams(**kwargs)


@jax.jit
def pallas_sequential_preLN__sliding_block_cached__glu_gated_swiglu__decode_kernel(
    A_x: jax.Array,
    A_k_cache: jax.Array,
    A_v_cache: jax.Array,
    A_wq: jax.Array,
    A_wo: jax.Array,
    B_x: jax.Array,
    B_w1: jax.Array,
    B_w3: jax.Array,
    B_w2: jax.Array,
):
    del B_x
    b, sq, d_model = A_x.shape
    hkv, sk = A_k_cache.shape[1], A_k_cache.shape[2]
    d_ff = B_w1.shape[1]
    assert b == 1 and sq == 1 and hkv == _HQ and A_k_cache.shape[3] == _DH
    win = min(4096, max(256, sk // 4))
    bf16, f32 = jnp.bfloat16, jnp.float32

    k_t = jnp.swapaxes(A_k_cache, 2, 3)
    v_t = jnp.swapaxes(A_v_cache, 2, 3)
    x2 = A_x.reshape(1, d_model)
    wo3 = A_wo.reshape(_HQ, _DH, d_model)

    dma = pltpu.SemaphoreType.DMA
    out = pl.pallas_call(
        functools.partial(_kernel, win_start=sk - win, win=win),
        out_shape=jax.ShapeDtypeStruct((1, d_model), A_x.dtype),
        in_specs=[pl.BlockSpec(memory_space=pl.ANY)] * 8,
        out_specs=pl.BlockSpec(memory_space=pltpu.VMEM),
        scratch_shapes=[
            pltpu.VMEM((1, d_model), bf16),
            pltpu.VMEM((_ROWS, d_model), bf16),
            pltpu.VMEM((2, d_model, _GRP * _DH), bf16),
            pltpu.VMEM((2, _DH, d_model), bf16),
            pltpu.VMEM((d_model, d_ff), bf16),
            pltpu.VMEM((d_model, d_ff), bf16),
            pltpu.VMEM((d_ff, d_model), bf16),
            pltpu.VMEM((2, _DH, win), bf16),
            pltpu.VMEM((2, _DH, win), bf16),
            pltpu.VMEM((2, _ROWS, _DH), bf16),
            pltpu.VMEM((_ROWS, win), f32),
            pltpu.VMEM((_ROWS, 128), f32),
            pltpu.VMEM((_ROWS, _DH), bf16),
            pltpu.VMEM((_ROWS, d_model), f32),
            dma((1,)), dma((2,)), dma((2,)), dma((2,)), dma((2,)),
            dma((_N_FFN_SEMS,)), dma((2 + _W2_HI // 128,)),
        ],
        compiler_params=_compiler_params(),
    )(x2, k_t, v_t, A_wq, wo3, B_w1, B_w3, B_w2)
    return out.reshape(b, sq, d_model)
```

```python
import dataclasses
import functools

import jax
import jax.numpy as jnp
import numpy as np
import jax.experimental.pallas as pl
import jax.experimental.pallas.tpu as pltpu

_HQ = 32
_DH = 192
_EPS = float(np.asarray(1e-5, dtype=jnp.bfloat16))
_SCALE = float(np.asarray(_DH ** -0.5, dtype=jnp.bfloat16))
_ROWS = 8
_PAIR = 2 * _DH
_GRP = 4
_HI, _LO = 0, 1

_KV_W = (384, 768, 640, 768, 768, 768)
_KV_R = 32
_RB = 8
_LOOK = 24
_PRE = 2
_N_SL = 8
_W2_HI = 256
_W2_VPU = 256
_LAND = 15
_N_FFN_SEMS = 18


def _rnd(x):
    return x.astype(jnp.bfloat16).astype(jnp.float32)


def _layernorm(x):
    m = jnp.mean(x, axis=-1, keepdims=True)
    c = x - m
    v = jnp.mean(c * c, axis=-1, keepdims=True)
    return _rnd(x - _rnd(m)) / _rnd(jnp.sqrt(_rnd(_rnd(v) + _EPS)))


def _kernel(x_hbm, k_hbm, v_hbm, wq_hbm, wo_hbm, w1_hbm, w3_hbm, w2_hbm, o_ref,
            x_v, xn_v, wq_v, wo_v, w1_v, w3_v, w2_v, kbuf, vbuf, q_v, s_v, m_v, av_v, res_v,
            sem_x, sem_wq, sem_k, sem_v, sem_wo, sem_lo, sem_hi,
            *, win_start, win):
    f32, bf16 = jnp.float32, jnp.bfloat16
    d_model = x_v.shape[-1]
    d_ff = w1_v.shape[-1]
    n_rb = _DH // _KV_R
    n = n_rb * len(_KV_W)
    n_wq = d_model // _RB // _GRP
    n_wo = 2 * (_DH // _RB)
    wo_cols = ((0, 256), (256, d_model - 256))
    sl = win // _N_SL
    assert sum(_KV_W) == win and n_wq + n_wo <= 2 * n and _LOOK <= n and n_wq % 2 == 0
    assert d_ff == 4 * _PAIR and d_model == 5 * 128 and _GRP * _DH == d_ff // 2

    def ds(start, size, align):
        if isinstance(start, int):
            return pl.ds(start, size)
        return pl.ds(pl.multiple_of(start, align), size)

    def kv_copy(hbm, buf, sem, h, slot, t):
        rows = pl.ds((t % n_rb) * _KV_R, _KV_R)
        c, w = sum(_KV_W[:t // n_rb]), _KV_W[t // n_rb]
        return pltpu.make_async_copy(
            hbm.at[0, h, rows, pl.ds(win_start + c, w)],
            buf.at[slot, rows, pl.ds(c, w)], sem.at[slot])

    k_copy = functools.partial(kv_copy, k_hbm, kbuf, sem_k)
    v_copy = functools.partial(kv_copy, v_hbm, vbuf, sem_v)

    def wq_copy(grp, slot, r0, nrows):
        rows = ds(r0, nrows, _RB)
        return pltpu.make_async_copy(
            wq_hbm.at[rows, ds(grp * (_GRP * _DH), _GRP * _DH, 128)],
            wq_v.at[slot, rows, :], sem_wq.at[slot])

    def wo_copy(h, slot, b):
        rows, cols = pl.ds((b // 2) * _RB, _RB), pl.ds(*wo_cols[b % 2])
        return pltpu.make_async_copy(wo_hbm.at[h, rows, cols], wo_v.at[slot, rows, cols],
                                     sem_wo.at[slot])

    def block_copy(hbm, buf, r0, nrows, c0, ncols, sem):
        rows, cols = ds(r0, nrows, _RB), pl.ds(c0, ncols)
        return pltpu.make_async_copy(hbm.at[rows, cols], buf.at[rows, cols], sem)

    def wait_all(ref, sem):
        pltpu.make_async_copy(ref, ref, sem).wait()

    w1_hi = d_model // 2
    w3_lo = d_model - d_model // 4
    mxu_end = d_ff - _W2_VPU
    w2_groups, r = [], _W2_HI
    while r < mxu_end:
        w2_groups.append((r, 256 if mxu_end - r >= 512 else 128))
        r += w2_groups[-1][1]
    g_w3, g_w2 = 1, 5
    g_vpu = g_w2 + len(w2_groups)
    lo1 = [(w1_hbm, w1_v, r, 16, 0, d_ff, 0) for r in range(w1_hi, d_model, 16)]
    lo3 = [(w3_hbm, w3_v, r, 16, 0, d_ff, g_w3 + r // 128) for r in range(0, w3_lo, 16)]
    mixed = sorted([(0.6 * (i + 0.5) / len(lo1), 0, i) for i in range(len(lo1))]
                   + [((i + 0.5) / len(lo3), 1, i) for i in range(len(lo3))])
    ffn_lo = ([(lo1, lo3)[which][i] for _, which, i in mixed]
              + [(w2_hbm, w2_v, r, 32, 0, d_model, g_w2 + gi)
                 for gi, (r0, nr) in enumerate(w2_groups) for r in range(r0, r0 + nr, 32)]
              + [(w2_hbm, w2_v, r, 32, 0, d_model, g_vpu + i)
                 for i, r in enumerate(range(mxu_end, d_ff, 32))])
    ffn_hi = ([(w3_hbm, w3_v, r, _RB, c, d_ff // 2, 1)
               for r in range(w3_lo, d_model, _RB) for c in (0, d_ff // 2)]
              + [(w2_hbm, w2_v, r, _RB, 0, d_model, 2 + r // 128)
                 for r in range(0, _W2_HI, _RB)])
    assert ffn_lo[-1][6] + 1 == _N_FFN_SEMS and len(ffn_hi) <= len(ffn_lo)

    def ffn_lo_copy(i):
        return block_copy(*ffn_lo[i][:6], sem_lo.at[ffn_lo[i][6]])

    def ffn_hi_copy(i):
        return block_copy(*ffn_hi[i][:6], sem_hi.at[ffn_hi[i][6]])

    pieces = sorted([((i + 0.5) / n_wq, "q", i) for i in range(n_wq)]
                    + [((i + 0.5) / n_wo, "o", i) for i in range(n_wo)])
    piece_at = {(i * 2 * n) // len(pieces): p[1:] for i, p in enumerate(pieces)}
    n_a = sum(1 for t in piece_at if t < n)

    def start_hi(j, kind, b):
        slot, quarter = j & 1, j & (_GRP - 1)
        grp = (j >> 2) + 1
        if kind == "o":
            wo_copy(j, slot, b).start(priority=_HI)
        elif isinstance(j, int):
            wq_copy(grp, grp & 1, (quarter * n_wq + b) * _RB, _RB).start(priority=_HI)
        else:
            @pl.when(j < _HQ - _GRP)
            def _():
                wq_copy(grp, grp & 1, (quarter * n_wq + b) * _RB, _RB).start(priority=_HI)

            @pl.when(j >= _HQ - _GRP)
            def _():
                block_copy(w1_hbm, w1_v, (quarter * (n_wq // 2) + b // 2) * _RB, _RB,
                           (b % 2) * (d_ff // 2), d_ff // 2,
                           sem_hi.at[0]).start(priority=_HI)

    def qk_slice(slot, i, mx):
        cols = pl.ds(i * sl, sl)
        s = jnp.dot(q_v[slot], kbuf[slot, :, cols], preferred_element_type=f32)
        s = _rnd(_rnd(s) * _SCALE)
        s_v[:, cols] = s
        for c in range(sl // 128):
            mx = jnp.maximum(mx, s[:, c * 128:(c + 1) * 128])
        return mx

    def pv_slice(slot, i, carry):
        acc, den = carry
        cols = pl.ds(i * sl, sl)
        p = jnp.exp(s_v[:, cols] - jnp.concatenate([m_v[...]] * (sl // 128), axis=-1))
        for c in range(sl // 128):
            den = den + p[:, c * 128:(c + 1) * 128]
        acc = acc + jax.lax.dot_general(
            p.astype(bf16), vbuf[slot, :, cols], (((1,), (1,)), ((), ())),
            preferred_element_type=f32)
        return acc, den

    def pv_init():
        return jnp.zeros((_ROWS, _DH), f32), jnp.zeros((_ROWS, 128), f32)

    def pv_finish(acc, den):
        return (acc / jnp.sum(den, axis=-1, keepdims=True)).astype(bf16)

    def out_proj(slot, o):
        wait_all(wo_v.at[slot], sem_wo.at[slot])
        return jnp.dot(o, wo_v[slot], preferred_element_type=f32)

    def q_proj(slot, half):
        w = wq_v[slot, :, ds(half * _PAIR, _PAIR, 128)]
        q = jnp.dot(xn_v[...], w, preferred_element_type=f32).astype(bf16)
        q_v[0] = q[:, :_DH]
        q_v[1] = q[:, _DH:]

    x_copy = pltpu.make_async_copy(x_hbm, x_v, sem_x.at[0])
    k0 = [k_copy(0, 0, t) for t in range(n)]
    wq0 = [wq_copy(0, 0, r, 32) for r in range(0, d_model, 32)]
    seq0 = [(k0, wq0)[which][i] for _, which, i in sorted(
        [((i + 0.5) / len(k0), 0, i) for i in range(len(k0))]
        + [((i + 0.5) / len(wq0), 1, i) for i in range(len(wq0))])]
    n0 = len(seq0)
    seq0 += [v_copy(0, 0, t) for t in range(_LOOK)]
    hi0 = [p[1:] for p in pieces[:n_a]]
    hi0_at = {(i * n0) // (n_a - _PRE): p for i, p in enumerate(hi0[_PRE:])}
    x_copy.start(priority=_HI)
    for c in seq0[:_LOOK]:
        c.start(priority=_LO)
    for p in hi0[:_PRE]:
        start_hi(0, *p)
    for t in range(n0):
        seq0[t].wait()
        if t in hi0_at:
            start_hi(0, *hi0_at[t])
        seq0[t + _LOOK].start(priority=_LO)
        if t == 2:
            x_copy.wait()
            x = jnp.broadcast_to(x_v[...].astype(f32), (_ROWS, d_model))
            xn_v[...] = _layernorm(x).astype(bf16)
            res_v[...] = jnp.zeros_like(x)
    q_proj(0, 0)

    gap = (n - 1) // _N_SL

    def phase(j, carry):
        slot = j & 1
        prev = 1 - slot
        gslot = (j >> 2) & 1
        quarter = j & (_GRP - 1)

        def tick(t):
            if t < n:
                k_copy(j, slot, t).wait()
            else:
                v_copy(j, slot, t - n).wait()
            if t in piece_at:
                start_hi(j, *piece_at[t])
            u = t + _LOOK
            if u < n:
                k_copy(j, slot, u).start(priority=_LO)
            elif u < 2 * n:
                v_copy(j, slot, u - n).start(priority=_LO)
            else:
                @pl.when(j + 1 < _HQ)
                def _():
                    k_copy(j + 1, prev, u - 2 * n).start(priority=_LO)

                @pl.when(j + 1 == _HQ)
                def _():
                    ffn_lo_copy(u - 2 * n).start(priority=_LO)

        @pl.when(j > 0)
        def _():
            pv = pv_init()
            for t in range(n):
                tick(t)
                if t % gap == 0 and t // gap < _N_SL:
                    pv = pv_slice(prev, t // gap, pv)
                if t == gap * _N_SL:
                    @pl.when(quarter == 0)
                    def _():
                        wait_all(wq_v.at[gslot], sem_wq.at[gslot])

                    @pl.when(slot == 0)
                    def _():
                        q_proj(gslot, quarter >> 1)
            av_v[...] = pv_finish(*pv)

        mx = jnp.full((_ROWS, 128), -jnp.inf, f32)
        for t in range(n):
            tick(n + t)
            if t % gap == 0 and t // gap < _N_SL:
                mx = qk_slice(slot, t // gap, mx)
            if t == gap * _N_SL:
                m_v[...] = jnp.broadcast_to(jnp.max(mx, axis=-1, keepdims=True), (_ROWS, 128))

                @pl.when(j > 0)
                def _():
                    res_v[...] += out_proj(prev, av_v[...])
        return carry

    jax.lax.fori_loop(0, _HQ, phase, 0)

    done = [0]

    def ticks_to(m):
        for i in range(done[0], m + 1):
            ffn_lo_copy(i).wait()
            if i < len(ffn_hi):
                ffn_hi_copy(i).start(priority=_HI)
            if i + _LOOK < len(ffn_lo):
                ffn_lo_copy(i + _LOOK).start(priority=_LO)
        done[0] = max(done[0], m + 1)

    def lo_done(group):
        return max(i for i, e in enumerate(ffn_lo) if e[6] == group)

    def hi_done(group):
        return max(i for i, e in enumerate(ffn_hi) if e[6] == group) + _LAND

    last = (_HQ - 1) & 1
    pv = pv_init()
    for i in range(_N_SL):
        ticks_to(i * 18 // _N_SL)
        pv = pv_slice(last, i, pv)
    ticks_to(18)
    hres = _rnd(x + _rnd(res_v[...] + out_proj(last, pv_finish(*pv))))
    ticks_to(21)
    hn = _layernorm(hres).astype(bf16)

    t0 = max(lo_done(0), 23)
    ticks_to(t0)
    wait_all(w1_v.at[pl.ds(0, w1_hi), :], sem_hi.at[0])
    gates = []
    for s in range(4):
        gates.append(jnp.dot(hn, w1_v[:, s * _PAIR:(s + 1) * _PAIR],
                             preferred_element_type=f32))
        ticks_to(t0 + (5 * (s + 1)) // 2)
    gate = _rnd(jnp.concatenate(gates, axis=-1))
    gate = _rnd(gate * jax.nn.sigmoid(gate))

    def up_chunk(c):
        return jnp.dot(hn[:, c * 128:(c + 1) * 128], w3_v[c * 128:(c + 1) * 128, :],
                       preferred_element_type=f32)

    up = None
    for c in range(3):
        ticks_to(lo_done(g_w3 + c))
        up = up_chunk(c) if up is None else up + up_chunk(c)
    ticks_to(max(hi_done(1) + 1, lo_done(g_w3 + 3)))
    wait_all(w3_v.at[pl.ds(w3_lo, d_model - w3_lo), :], sem_hi.at[1])
    up = up + up_chunk(3) + up_chunk(4)
    act = (gate * _rnd(up)).astype(bf16)

    def down(r0, nr):
        return jnp.dot(act[:, r0:r0 + nr], w2_v[r0:r0 + nr, :], preferred_element_type=f32)

    act_col = jnp.concatenate(
        [jnp.broadcast_to(act[0:1, c:c + 128].astype(f32), (128, 128)).T
         for c in range(mxu_end, d_ff, 128)], axis=0)

    out = jnp.zeros_like(hres)
    pending = list(range(_W2_HI // 128))
    for gi, (r0, nr) in enumerate(w2_groups):
        ticks_to(lo_done(g_w2 + gi))
        part = down(r0, nr)
        while pending and (hi_done(2 + pending[0]) <= lo_done(g_w2 + gi)
                           or gi == len(w2_groups) - 1):
            c = pending.pop(0)
            wait_all(w2_v.at[pl.ds(c * 128, 128), :], sem_hi.at[2 + c])
            part = part + down(c * 128, 128)
        out = out + part

    tail = jnp.zeros((8, d_model), f32)
    for i, r in enumerate(range(mxu_end, d_ff, 32)):
        ticks_to(lo_done(g_vpu + i))
        a = act_col[r - mxu_end:r - mxu_end + 32, :]
        prod = w2_v[r:r + 32, :].astype(f32) * jnp.concatenate([a] * (d_model // 128), axis=-1)
        for k in range(4):
            tail = tail + prod[k * 8:(k + 1) * 8, :]
    assert done[0] == len(ffn_lo)
    ffn = out[0:1, :] + jnp.sum(tail, axis=0, keepdims=True)
    o_ref[...] = (hres[0:1, :] + _rnd(ffn)).astype(o_ref.dtype)


def _compiler_params():
    kwargs = dict(vmem_limit_bytes=48 * 1024 * 1024)
    if any(f.name == "disable_semaphore_checks" for f in dataclasses.fields(pltpu.CompilerParams)):
        kwargs["disable_semaphore_checks"] = True
    return pltpu.CompilerParams(**kwargs)


@jax.jit
def pallas_sequential_preLN__sliding_block_cached__glu_gated_swiglu__decode_kernel(
    A_x: jax.Array,
    A_k_cache: jax.Array,
    A_v_cache: jax.Array,
    A_wq: jax.Array,
    A_wo: jax.Array,
    B_x: jax.Array,
    B_w1: jax.Array,
    B_w3: jax.Array,
    B_w2: jax.Array,
):
    del B_x
    b, sq, d_model = A_x.shape
    hkv, sk = A_k_cache.shape[1], A_k_cache.shape[2]
    d_ff = B_w1.shape[1]
    assert b == 1 and sq == 1 and hkv == _HQ and A_k_cache.shape[3] == _DH
    win = min(4096, max(256, sk // 4))
    bf16, f32 = jnp.bfloat16, jnp.float32

    k_t = jnp.swapaxes(A_k_cache, 2, 3)
    v_t = jnp.swapaxes(A_v_cache, 2, 3)
    x2 = A_x.reshape(1, d_model)
    wo3 = A_wo.reshape(_HQ, _DH, d_model)

    dma = pltpu.SemaphoreType.DMA
    out = pl.pallas_call(
        functools.partial(_kernel, win_start=sk - win, win=win),
        out_shape=jax.ShapeDtypeStruct((1, d_model), A_x.dtype),
        in_specs=[pl.BlockSpec(memory_space=pl.ANY)] * 8,
        out_specs=pl.BlockSpec(memory_space=pltpu.VMEM),
        scratch_shapes=[
            pltpu.VMEM((1, d_model), bf16),
            pltpu.VMEM((_ROWS, d_model), bf16),
            pltpu.VMEM((2, d_model, _GRP * _DH), bf16),
            pltpu.VMEM((2, _DH, d_model), bf16),
            pltpu.VMEM((d_model, d_ff), bf16),
            pltpu.VMEM((d_model, d_ff), bf16),
            pltpu.VMEM((d_ff, d_model), bf16),
            pltpu.VMEM((2, _DH, win), bf16),
            pltpu.VMEM((2, _DH, win), bf16),
            pltpu.VMEM((2, _ROWS, _DH), bf16),
            pltpu.VMEM((_ROWS, win), f32),
            pltpu.VMEM((_ROWS, 128), f32),
            pltpu.VMEM((_ROWS, _DH), bf16),
            pltpu.VMEM((_ROWS, d_model), f32),
            dma((1,)), dma((2,)), dma((2,)), dma((2,)), dma((2,)),
            dma((_N_FFN_SEMS,)), dma((2 + _W2_HI // 128,)),
        ],
        compiler_params=_compiler_params(),
    )(x2, k_t, v_t, A_wq, wo3, B_w1, B_w3, B_w2)
    return out.reshape(b, sq, d_model)
```
